```python
import jax
import jax.numpy as jnp

def _softmax(x, axis=-1):
    return jax.nn.softmax(x, axis=axis)
def _gelu(x):
    return jax.nn.gelu(x, approximate=True)
def _silu(x):
    return jax.nn.silu(x)
def _sigmoid(x):
    return jax.nn.sigmoid(x)
def _layernorm(x, axis=-1, eps=1e-5):
    m = jnp.mean(x, axis=axis, keepdims=True)
    v = jnp.var(x, axis=axis, keepdims=True)
    return (x - m) / jnp.sqrt(v + eps)
def _scatter_add(tgt, idx, src, axis=0):
    return tgt.at[idx].add(src)
def _segment_sum(src, seg, n):
    return jax.ops.segment_sum(src, seg, n)
class _Rng:
    def __init__(self, key):
        self._k = key
    def _next(self):
        self._k, sub = jax.random.split(self._k)
        return sub
    def normal(self, shape):
        return jax.random.normal(self._next(), shape, dtype=jnp.bfloat16)
    def randint(self, lo, hi, shape):
        return jax.random.randint(self._next(), shape, lo, hi, dtype=jnp.int32)
    def uniform(self, shape, lo=0.0, hi=1.0):
        return jax.random.uniform(self._next(), shape, jnp.bfloat16, lo, hi)
    def permutation(self, n):
        return jax.random.permutation(self._next(), n)


kernel_name = 'gated_mix__compressed_kv_cla__ssm_conv_h3__prompt'

def setup_inputs():
    _rng = _Rng(jax.random.key(int.from_bytes(__import__("os").urandom(4), "little")))
    _w = (lambda a: (lambda t: t.astype(jnp.bfloat16) if jnp.issubdtype(t.dtype, jnp.floating) else t)(jnp.asarray(a)))
    def _A_setup():
        B, H, Sq, Sk, D, M = 1, 32, 2048, 2048, 128, 1024
        Dc = 4 * D
        return {
            "x": _w((lambda *s: _rng.normal(s) * 0.05)(B, Sq, M)),
            "c_kv": _w((lambda *s: _rng.normal(s) * 0.05)(B, Sk, Dc)),
            "w_q": _w((lambda *s: _rng.normal(s) * 0.05)(M, H, D) * (M ** -0.5)),
            "w_uk": _w((lambda *s: _rng.normal(s) * 0.05)(Dc, H, D) * (Dc ** -0.5)),
            "w_uv": _w((lambda *s: _rng.normal(s) * 0.05)(Dc, H, D) * (Dc ** -0.5)),
            "w_o": _w((lambda *s: _rng.normal(s) * 0.05)(H, D, M) * ((H * D) ** -0.5)),
        }
    _A_in = _A_setup()

    def _B_setup():
        B, S, D = 1, 2048, 1024
        ks = 4
        return {
            "q": _w((lambda *s: _rng.normal(s) * 0.05)(B, S, D)),
            "k": _w((lambda *s: _rng.normal(s) * 0.05)(B, S, D)),
            "v": _w((lambda *s: _rng.normal(s) * 0.05)(B, S, D)),
            "shift_k": _w((lambda *s: _rng.normal(s) * 0.05)(D, ks) * 0.5),
            "ssm_k": _w((lambda *s: _rng.normal(s) * 0.05)(D, S) * (1.0 / S ** 0.5)),
            "ssm_D": _w((lambda *s: _rng.normal(s) * 0.05)(D)),
        }
    _B_in = _B_setup()

    return {
        "A_x": _A_in["x"],
        "A_c_kv": _A_in["c_kv"],
        "A_w_q": _A_in["w_q"],
        "A_w_uk": _A_in["w_uk"],
        "A_w_uv": _A_in["w_uv"],
        "A_w_o": _A_in["w_o"],
        "B_q": _B_in["q"],
        "B_k": _B_in["k"],
        "B_v": _B_in["v"],
        "B_shift_k": _B_in["shift_k"],
        "B_ssm_k": _B_in["ssm_k"],
        "B_ssm_D": _B_in["ssm_D"],
        "gate_w": _w((lambda *s: _rng.normal(s) * 0.05)(1024)),
    }

def reference(A_x, A_c_kv, A_w_q, A_w_uk, A_w_uv, A_w_o, B_q, B_k, B_v, B_shift_k, B_ssm_k, B_ssm_D, gate_w):
    def _A_ref(x, c_kv, w_q, w_uk, w_uv, w_o):
        B, Sq, M = x.shape[0], x.shape[1], x.shape[2]
        Sk = c_kv.shape[1]
        H, D = w_q.shape[1], w_q.shape[2]
        q = jnp.einsum("bqm,mhd->bhqd", x, w_q)
        k = jnp.einsum("bkc,chd->bhkd", c_kv, w_uk)
        v = jnp.einsum("bkc,chd->bhkd", c_kv, w_uv)
        scores = jnp.einsum("bhqd,bhkd->bhqk", q, k) * (D ** -0.5)
        off = Sk - Sq
        qi = jnp.arange(Sq)[:, None]
        kj = jnp.arange(Sk)[None, :]
        cmask = kj <= (qi + off)
        scores = jnp.where(cmask[None, None], scores, -1e9)
        p = _softmax(scores, axis=-1)
        ctx = jnp.einsum("bhqk,bhkd->bhqd", p, v)
        return jnp.einsum("bhqd,hdm->bqm", ctx, w_o)

    def _B_ref(q, k, v, shift_k, ssm_k, ssm_D):
        B, S, D = q.shape
        ks = shift_k.shape[-1]
        k_pad = jnp.pad(k, ((0, 0), (ks - 1, 0), (0, 0)))
        k_shift = jnp.zeros_like(k)
        for t in range(ks):
            k_shift = k_shift + k_pad[:, t:t + S, :] * shift_k[:, ks - 1 - t][None, None, :]
        kv = k_shift * v
        L = 2 * S
        kv_pad = jnp.pad(kv, ((0, 0), (0, S), (0, 0)))
        kf_pad = jnp.pad(ssm_k, ((0, 0), (0, S)))
        kv_f = (lambda x, axes=(-2,-1): jnp.fft.rfft2(x.astype(jnp.float32), axes=axes))(kv_pad[:, None, :, :], axes=(1, 2))
        kf_f = (lambda x, axes=(-2,-1): jnp.fft.rfft2(x.astype(jnp.float32), axes=axes))(kf_pad[:, None, :], axes=(1, 2))
        kf_f = (lambda x, *d: x.transpose(*d))(kf_f, 1, 2, 0)
        y_f = kv_f * kf_f[None, :, :, :]
        y = (lambda x, s, axes=(-2,-1): jnp.fft.irfft2(x, s=s, axes=axes).astype(jnp.bfloat16))(y_f, (1, L), axes=(1, 2))[:, 0, :S, :]
        y = y + kv * ssm_D[None, None, :]
        return q * y

    x = A_x
    g = _sigmoid((x * gate_w).sum(-1, keepdims=True))
    a = _A_ref(x, A_c_kv, A_w_q, A_w_uk, A_w_uv, A_w_o)
    b = _B_ref(x, B_k, B_v, B_shift_k, B_ssm_k, B_ssm_D)
    return g * a + (1 - g) * b
```

```python
import math

import jax
import jax.numpy as jnp
from jax import lax
import jax.experimental.pallas as pl
import jax.experimental.pallas.tpu as pltpu

F32 = jnp.float32
BF16 = jnp.bfloat16

S = 2048
M = 1024
H = 32
D = 128
DC = 512
HG = 8
NG = H // HG
RC = 512
NRC = S // RC
BQ = 128
NBQ = S // BQ
CB = 128
NCB = S // CB
NCG = M // 128
FO = 256
NEG = -1e9
NT = (((1,), (1,)), ((), ()))
QSCALE = (D ** -0.5) * math.log2(math.e)


def _dft_mats():
    shp = (2, 128, 128)
    hf = lax.broadcasted_iota(jnp.int32, shp, 0)
    r = lax.broadcasted_iota(jnp.int32, shp, 1)
    j = lax.broadcasted_iota(jnp.int32, shp, 2)
    f = hf * 64 + (r & 63)
    k = ((2 * f + 1) * j + jnp.where(r >= 64, 128, 0)) & 511
    fm = jnp.cos(k.astype(F32) * (2 * math.pi / 512))
    ff = hf * 64 + (j & 63)
    k2 = ((2 * ff + 1) * (r + 128) + jnp.where(j >= 64, 128, 0)) & 511
    gm = jnp.cos(k2.astype(F32) * (2 * math.pi / 512)) * (1.0 / 128)
    return fm.astype(BF16), gm.astype(BF16)


def _kernel(x_h, c_h, wq_h, wuk_h, wuv_h, wo_h, bk_h, bv_h, sk_h, h_h, d_h, gw_h,
            o_h,
            x_v, c_v, wq_raw, wuk_raw, wuv_raw, wo_v, bk_s, bv_s, sk_v, h_s, d_v, gw_v,
            wq_s, wkv_s, q_s, k_s, v_s, ctx_s, kv_s, y_s, u_s, ht_s, f_s, g_s, o_s,
            sem_c, sem_x, sem_wq, sem_wuk, sem_wuv, sem_wo, sem_bk, sem_bv,
            sem_h, sem_small, sem_o):
    def cp_c(b):
        return pltpu.make_async_copy(c_h.at[pl.ds(b * RC, RC)], c_v.at[pl.ds(b * RC, RC)], sem_c.at[b])

    def cp_x(b):
        return pltpu.make_async_copy(x_h.at[pl.ds(b * RC, RC)], x_v.at[pl.ds(b * RC, RC)], sem_x.at[b])

    def cp_wq(g, b):
        rows = pl.ds(b * 256, 256)
        return pltpu.make_async_copy(wq_h.at[rows, g], wq_raw.at[g, rows], sem_wq.at[g * 4 + b])

    def cp_wuk(g, b):
        rows = pl.ds(b * 128, 128)
        return pltpu.make_async_copy(wuk_h.at[rows, g], wuk_raw.at[g, rows], sem_wuk.at[g * 4 + b])

    def cp_wuv(g, b):
        rows = pl.ds(b * 128, 128)
        return pltpu.make_async_copy(wuv_h.at[rows, g], wuv_raw.at[g, rows], sem_wuv.at[g * 4 + b])

    def cp_b(src, dst, sem, p):
        cg = p // 2
        rows = pl.ds((p % 2) * 1024, 1024)
        return pltpu.make_async_copy(src.at[rows, pl.ds(cg * 128, 128)], dst.at[cg, rows], sem.at[p])

    def cp_h(cg):
        return pltpu.make_async_copy(h_h.at[pl.ds(cg * 128, 128)], h_s.at[cg], sem_h.at[cg])

    cp_wo = pltpu.make_async_copy(wo_h, wo_v, sem_wo.at[0])
    cp_small = [pltpu.make_async_copy(sk_h, sk_v, sem_small.at[0]),
                pltpu.make_async_copy(d_h, d_v, sem_small.at[1]),
                pltpu.make_async_copy(gw_h, gw_v, sem_small.at[2])]

    def cp_o(r):
        rows = pl.ds(r * FO, FO)
        return pltpu.make_async_copy(o_s.at[rows], o_h.at[rows], sem_o.at[r])

    def start_group(g):
        for b in range(4):
            cp_wq(g, b).start()
            cp_b(bk_h, bk_s, sem_bk, g * 4 + b).start()
            cp_b(bv_h, bv_s, sem_bv, g * 4 + b).start()
        cp_h(2 * g).start()
        cp_h(2 * g + 1).start()

    def start_wkv(g):
        for b in range(4):
            cp_wuk(g, b).start()
            cp_wuv(g, b).start()

    start_wkv(0)
    cp_c(0).start()
    for cp in cp_small:
        cp.start()
    cp_wq(0, 0).start()
    cp_b(bk_h, bk_s, sem_bk, 0).start()
    cp_b(bv_h, bv_s, sem_bv, 0).start()
    for b in range(1, 4):
        cp_c(b).start()
        cp_wq(0, b).start()
        cp_b(bk_h, bk_s, sem_bk, b).start()
        cp_b(bv_h, bv_s, sem_bv, b).start()
    for b in range(4):
        cp_x(b).start()
    cp_h(0).start()
    cp_h(1).start()

    fm, gm = _dft_mats()
    f_s[...] = fm
    g_s[...] = gm

    def relayout_wkv(g, b):
        rows = pl.ds(pl.multiple_of(b * 128, 128), 128)
        tk = jnp.swapaxes(wuk_raw[g, rows], 0, 1)
        tv = jnp.swapaxes(wuv_raw[g, rows], 0, 1)
        for hh in range(HG):
            wkv_s[rows, hh * 128:(hh + 1) * 128] = tk[hh]
            wkv_s[rows, 1024 + hh * 128:1024 + (hh + 1) * 128] = tv[hh]

    for b in range(4):
        cp_wuk(0, b).wait()
        cp_wuv(0, b).wait()
        relayout_wkv(0, b)
    for cp in cp_small:
        cp.wait()

    def group_body(g, carry):
        @pl.when(g + 1 < NG)
        def _():
            start_wkv(g + 1)
            start_group(g + 1)

        @pl.when(g == 1)
        def _():
            cp_wo.start()

        def kv_body(b, c2):
            @pl.when(g == 0)
            def _():
                cp_c(b).wait()
            p = g * 4 + b
            cp_wq(g, b).wait()
            cp_b(bk_h, bk_s, sem_bk, p).wait()
            cp_b(bv_h, bv_s, sem_bv, p).wait()

            rows = pl.ds(pl.multiple_of(b * RC, RC), RC)
            kk = jnp.dot(c_v[rows, :], wkv_s[...], preferred_element_type=F32)
            for hh in range(HG):
                k_s[hh, rows, :] = kk[:, hh * 128:(hh + 1) * 128].astype(BF16)
                v_s[hh, rows, :] = kk[:, 1024 + hh * 128:1024 + (hh + 1) * 128].astype(BF16)

            mrows = pl.ds(pl.multiple_of(b * 256, 256), 256)
            tq = jnp.swapaxes(wq_raw[g, mrows], 0, 1)
            for hh in range(HG):
                wq_s[mrows, hh * 128:(hh + 1) * 128] = tq[hh]

            cg = p // 2
            rh = p % 2
            row0 = pl.multiple_of(rh * 1024, 1024)
            kc = bk_s[cg, pl.ds(row0, 1024), :].astype(F32)
            prev = bk_s[cg, pl.ds(pl.multiple_of(jnp.maximum(row0 - 16, 0), 16), 16), :].astype(F32)
            prev = jnp.where(rh > 0, prev, 0.0)
            kk2 = jnp.concatenate([prev[8:], kc], axis=0)
            w = sk_v[:, pl.ds(pl.multiple_of(cg * 128, 128), 128)].astype(F32)
            acc = kc * w[0:1]
            for j in range(1, 4):
                acc = acc + pltpu.roll(kk2, j, axis=0)[8:] * w[j:j + 1]
            kvv = acc * bv_s[cg, pl.ds(row0, 1024), :].astype(F32)
            kv_s[cg, pl.ds(row0, 1024), :] = kvv.astype(BF16)
            return c2

        lax.fori_loop(0, NRC, kv_body, 0)

        def q_body(b, c2):
            @pl.when(g == 0)
            def _():
                cp_x(b).wait()
            p = g * 4 + b
            cg = p // 2
            hf = p % 2

            @pl.when(hf == 0)
            def _():
                cp_h(cg).wait()

            @pl.when(g + 1 < NG)
            def _():
                cp_wuk(g + 1, b).wait()
                cp_wuv(g + 1, b).wait()

            rows = pl.ds(pl.multiple_of(b * RC, RC), RC)
            qq = jnp.dot(x_v[rows, :], wq_s[...], preferred_element_type=F32) * QSCALE
            for hh in range(HG):
                q_s[hh, rows, :] = qq[:, hh * 128:(hh + 1) * 128].astype(BF16)

            relayout_wkv(jnp.minimum(g + 1, NG - 1), b)

            fh = f_s[hf]
            gh = g_s[hf]
            ucat = jnp.concatenate(
                [kv_s[cg, i * CB:(i + 1) * CB, :] for i in range(NCB)], axis=1)
            u_s[...] = jnp.dot(fh, ucat, preferred_element_type=F32)
            hcat = jnp.concatenate(
                [h_s[cg, :, m * CB:(m + 1) * CB] for m in range(NCB)], axis=0)
            hh_ = lax.dot_general(fh, hcat, NT, preferred_element_type=F32)
            sgn = jnp.where((lax.broadcasted_iota(jnp.int32, (64, 128), 0) & 1) == 0,
                            1.0, -1.0).astype(F32)
            for m in range(NCB):
                hr = hh_[0:64, m * CB:(m + 1) * CB]
                hi = hh_[64:128, m * CB:(m + 1) * CB]
                tr = sgn * hi
                ti = -(sgn * hr)
                if m > 0:
                    tr = tr + hh_[0:64, (m - 1) * CB:m * CB]
                    ti = ti + hh_[64:128, (m - 1) * CB:m * CB]
                ht_s[0:64, m * CB:(m + 1) * CB] = tr
                ht_s[64:128, m * CB:(m + 1) * CB] = ti
            RB = 32
            ys = []
            for i in range(NCB):
                yr_l = []
                yi_l = []
                for rb in range(0, 64, RB):
                    yr = None
                    yi = None
                    for m in range(i + 1):
                        a0 = (i - m) * CB
                        b0 = m * CB
                        ur = u_s[rb:rb + RB, a0:a0 + CB]
                        ui = u_s[64 + rb:64 + rb + RB, a0:a0 + CB]
                        hr = ht_s[rb:rb + RB, b0:b0 + CB]
                        hi = ht_s[64 + rb:64 + rb + RB, b0:b0 + CB]
                        pr = ur * hr - ui * hi
                        pi = ur * hi + ui * hr
                        yr = pr if yr is None else yr + pr
                        yi = pi if yi is None else yi + pi
                    yr_l.append(yr.astype(BF16))
                    yi_l.append(yi.astype(BF16))
                ys.append(jnp.concatenate(yr_l + yi_l, axis=0))
            ycat = jnp.concatenate(ys, axis=1)
            yo = jnp.dot(gh, ycat, preferred_element_type=F32)
            for i in range(NCB):
                old = jnp.where(hf == 0, 0.0, y_s[cg, i * CB:(i + 1) * CB, :])
                y_s[cg, i * CB:(i + 1) * CB, :] = old + yo[:, i * CB:(i + 1) * CB]
            return c2

        lax.fori_loop(0, NRC, q_body, 0)

        mask = (lax.broadcasted_iota(jnp.int32, (BQ, BQ), 1)
                <= lax.broadcasted_iota(jnp.int32, (BQ, BQ), 0))

        def attn_body(t, c2):
            def qk(hh, i):
                L = (i + 1) * BQ
                return lax.dot_general(q_s[hh, i * BQ:(i + 1) * BQ, :], k_s[hh, 0:L, :], NT,
                                       preferred_element_type=F32)

            def sm(i, s):
                L = (i + 1) * BQ
                sd = jnp.where(mask, s[:, L - BQ:], NEG)
                s = jnp.concatenate([s[:, :L - BQ], sd], axis=1) if i > 0 else sd
                m = jnp.max(s, axis=1, keepdims=True)
                p = jnp.exp2(s - m)
                l = jnp.sum(p, axis=1, keepdims=True)
                return p.astype(BF16), l

            def pv(hh, i, p, l):
                L = (i + 1) * BQ
                ctx = jnp.dot(p, v_s[hh, 0:L, :], preferred_element_type=F32)
                r = pl.reciprocal(l, approx=True)
                r = r * (2.0 - l * r)
                ctx_s[g * HG + hh, i * BQ:(i + 1) * BQ, :] = (ctx * r).astype(BF16)

            order = [(2 * t + u, i) for i in range(NBQ)[::-1] for u in range(2)]
            s_next = qk(*order[0])
            for n, (hh, i) in enumerate(order):
                s = s_next
                if n + 1 < len(order):
                    s_next = qk(*order[n + 1])
                p, l = sm(i, s)
                pv(hh, i, p, l)
            return c2

        lax.fori_loop(0, HG // 2, attn_body, 0)
        return carry

    lax.fori_loop(0, NG, group_body, 0)

    cp_wo.wait()

    def out_body(r, carry):
        rows = pl.ds(pl.multiple_of(r * FO, FO), FO)
        ctx = jnp.concatenate([ctx_s[hh, rows, :] for hh in range(H)], axis=1)
        a = jnp.dot(ctx, wo_v[...], preferred_element_type=F32)
        xf = x_v[rows, :].astype(F32)
        gw = gw_v[...].astype(F32)[None, :]
        gate = jax.nn.sigmoid(jnp.sum(xf * gw, axis=1, keepdims=True))
        dd = d_v[...].astype(F32)[None, :]
        for cg in range(NCG):
            cols = slice(cg * 128, (cg + 1) * 128)
            yb = y_s[cg, rows, :] + kv_s[cg, rows, :].astype(F32) * dd[:, cols]
            o_s[rows, cols] = (gate * a[:, cols] + (1.0 - gate) * (xf[:, cols] * yb)).astype(BF16)
        cp_o(r).start()
        return carry

    lax.fori_loop(0, S // FO, out_body, 0)
    for r in range(S // FO):
        cp_o(r).wait()


@jax.jit
def pallas_gated_mix__compressed_kv_cla__ssm_conv_h3__prompt_kernel(
    A_x: jax.Array,
    A_c_kv: jax.Array,
    A_w_q: jax.Array,
    A_w_uk: jax.Array,
    A_w_uv: jax.Array,
    A_w_o: jax.Array,
    B_q: jax.Array,
    B_k: jax.Array,
    B_v: jax.Array,
    B_shift_k: jax.Array,
    B_ssm_k: jax.Array,
    B_ssm_D: jax.Array,
    gate_w: jax.Array,
):
    del B_q
    x = A_x.reshape(S, M)
    c = A_c_kv.reshape(S, DC)
    wq = A_w_q.reshape(M, NG, HG, D)
    wuk = A_w_uk.reshape(DC, NG, HG, D)
    wuv = A_w_uv.reshape(DC, NG, HG, D)
    wo = A_w_o.reshape(H * D, M)
    bk = B_k.reshape(S, M)
    bv = B_v.reshape(S, M)
    skt = B_shift_k.T

    dma = pltpu.SemaphoreType.DMA
    scratch = [
        pltpu.VMEM((S, M), BF16),
        pltpu.VMEM((S, DC), BF16),
        pltpu.VMEM((NG, M, HG, D), BF16),
        pltpu.VMEM((NG, DC, HG, D), BF16),
        pltpu.VMEM((NG, DC, HG, D), BF16),
        pltpu.VMEM((H * D, M), BF16),
        pltpu.VMEM((NCG, S, 128), BF16),
        pltpu.VMEM((NCG, S, 128), BF16),
        pltpu.VMEM((4, M), BF16),
        pltpu.VMEM((NCG, 128, S), BF16),
        pltpu.VMEM((M,), BF16),
        pltpu.VMEM((M,), BF16),
        pltpu.VMEM((M, HG * D), BF16),
        pltpu.VMEM((DC, 2 * HG * D), BF16),
        pltpu.VMEM((HG, S, D), BF16),
        pltpu.VMEM((HG, S, D), BF16),
        pltpu.VMEM((HG, S, D), BF16),
        pltpu.VMEM((H, S, D), BF16),
        pltpu.VMEM((NCG, S, 128), BF16),
        pltpu.VMEM((NCG, S, 128), F32),
        pltpu.VMEM((128, S), F32),
        pltpu.VMEM((128, S), F32),
        pltpu.VMEM((2, 128, 128), BF16),
        pltpu.VMEM((2, 128, 128), BF16),
        pltpu.VMEM((S, M), BF16),
        dma((4,)), dma((4,)), dma((16,)), dma((16,)), dma((16,)), dma((1,)),
        dma((16,)), dma((16,)), dma((8,)), dma((3,)), dma((S // FO,)),
    ]
    out = pl.pallas_call(
        _kernel,
        out_shape=jax.ShapeDtypeStruct((S, M), BF16),
        in_specs=[pl.BlockSpec(memory_space=pl.ANY)] * 12,
        out_specs=pl.BlockSpec(memory_space=pl.ANY),
        scratch_shapes=scratch,
        compiler_params=pltpu.CompilerParams(vmem_limit_bytes=120 * 1024 * 1024),
    )(x, c, wq, wuk, wuv, wo, bk, bv, skt, B_ssm_k, B_ssm_D, gate_w)
    return out.reshape(1, S, M)
```

```python
import math

import jax
import jax.numpy as jnp
from jax import lax
import jax.experimental.pallas as pl
import jax.experimental.pallas.tpu as pltpu

F32 = jnp.float32
BF16 = jnp.bfloat16

S = 2048
M = 1024
H = 32
D = 128
DC = 512
HG = 8
NG = H // HG
RC = 512
NRC = S // RC
BQ = 128
NBQ = S // BQ
CB = 128
NCB = S // CB
NCG = M // 128
FO = 256
PADK = 16
NEG = -1e9
NT = (((1,), (1,)), ((), ()))
QSCALE = (D ** -0.5) * math.log2(math.e)


def _dft_mats():
    shp = (2, 128, 128)
    hf = lax.broadcasted_iota(jnp.int32, shp, 0)
    r = lax.broadcasted_iota(jnp.int32, shp, 1)
    j = lax.broadcasted_iota(jnp.int32, shp, 2)
    f = hf * 64 + (r & 63)
    k = ((2 * f + 1) * j + jnp.where(r >= 64, 128, 0)) & 511
    fm = jnp.cos(k.astype(F32) * (2 * math.pi / 512))
    ff = hf * 64 + (j & 63)
    k2 = ((2 * ff + 1) * (r + 128) + jnp.where(j >= 64, 128, 0)) & 511
    gm = jnp.cos(k2.astype(F32) * (2 * math.pi / 512)) * (1.0 / 128)
    return fm.astype(BF16), gm.astype(BF16)


U32 = jnp.uint32


def _pk(v):
    return pltpu.bitcast(v, U32)


def _up(v):
    return pltpu.bitcast(v, BF16)


def _own_block(trips, fn):
    def body(_, c):
        fn()
        return c
    lax.fori_loop(0, trips, body, 0)


def _spread(pieces, aux):
    n = len(pieces)
    done = 0
    for k, piece in enumerate(pieces):
        piece()
        tgt = (len(aux) * (k + 1)) // n
        while done < tgt:
            aux[done]()
            done += 1


def _kernel(x_h, c_h, wq_h, wuk_h, wuv_h, wo_h, bk_h, bv_h, sk_h, h_h, d_h, gw_h,
            o_h,
            x_v, c_v, wq_raw, wuk_raw, wuv_raw, wo_v, bk_s, bv_s, h_s,
            x_p, c_p, wq_s, wkv_s, q_s, k_s, v_s, ctx_s, kv_s, y_s, u_s, ht_s, f_s, g_s, o_s,
            sk_v, d_v, gw_v,
            sem_c, sem_x, sem_wq, sem_wuk, sem_wuv, sem_wo, sem_bk, sem_bv,
            sem_h, sem_small, sem_o):
    def cp_c(b):
        return pltpu.make_async_copy(c_h.at[pl.ds(b * RC, RC)], c_v.at[pl.ds(b * RC, RC)], sem_c.at[b])

    def cp_x(b):
        return pltpu.make_async_copy(x_h.at[pl.ds(b * RC, RC)], x_v.at[pl.ds(b * RC, RC)], sem_x.at[b])

    def cp_wq(g, b):
        rows = pl.ds(b * 256, 256)
        return pltpu.make_async_copy(wq_h.at[rows, g], wq_raw.at[g, rows], sem_wq.at[g * 4 + b])

    def cp_wuk(g, b):
        rows = pl.ds(b * 128, 128)
        return pltpu.make_async_copy(wuk_h.at[rows, g], wuk_raw.at[g, rows], sem_wuk.at[g * 4 + b])

    def cp_wuv(g, b):
        rows = pl.ds(b * 128, 128)
        return pltpu.make_async_copy(wuv_h.at[rows, g], wuv_raw.at[g, rows], sem_wuv.at[g * 4 + b])

    def cp_bk(p):
        cg = p // 2
        r0 = (p % 2) * 1024
        return pltpu.make_async_copy(bk_h.at[pl.ds(r0, 1024), pl.ds(cg * 128, 128)],
                                     bk_s.at[cg, pl.ds(PADK + r0, 1024)], sem_bk.at[p])

    def cp_bv(p):
        cg = p // 2
        rows = pl.ds((p % 2) * 1024, 1024)
        return pltpu.make_async_copy(bv_h.at[rows, pl.ds(cg * 128, 128)], bv_s.at[cg, rows], sem_bv.at[p])

    def cp_h(cg):
        return pltpu.make_async_copy(h_h.at[pl.ds(cg * 128, 128)], h_s.at[cg], sem_h.at[cg])

    cp_wo = pltpu.make_async_copy(wo_h, wo_v, sem_wo.at[0])
    cp_small = [pltpu.make_async_copy(sk_h, sk_v, sem_small.at[0]),
                pltpu.make_async_copy(d_h, d_v, sem_small.at[1]),
                pltpu.make_async_copy(gw_h, gw_v, sem_small.at[2])]

    def cp_o(r):
        rows = pl.ds(r * FO, FO)
        return pltpu.make_async_copy(o_s.at[rows], o_h.at[rows], sem_o.at[r])

    def start_kvaux(g, b):
        cp_wq(g, b).start()
        cp_bk(g * 4 + b).start()
        cp_bv(g * 4 + b).start()

    def start_wkv(g):
        for b in range(4):
            cp_wuk(g, b).start()
            cp_wuv(g, b).start()

    def relayout_wkv_step(g, b, s, which):
        m0 = pl.multiple_of(b * 128 + s * 32, 32)
        src = wuk_raw if which == 0 else wuv_raw
        t = jnp.swapaxes(src[g, pl.ds(m0, 32)], 0, 1)
        prow = pl.ds(pl.multiple_of(b * 64 + s * 16, 16), 16)
        for hh in range(HG):
            c0 = hh * 256 + which * 128
            wkv_s[prow, c0:c0 + 128] = _pk(t[hh])

    def stage_c(bn, rb):
        c_p[rb * 64:(rb + 1) * 64, :] = _pk(c_v[pl.ds(pl.multiple_of(bn * RC + rb * 128, 128), 128), :])

    def stage_x(bn, rb):
        x_p[rb * 64:(rb + 1) * 64, :] = _pk(x_v[pl.ds(pl.multiple_of(bn * RC + rb * 128, 128), 128), :])

    start_wkv(0)
    cp_c(0).start()

    fm, gm = _dft_mats()
    for hf in range(2):
        f_s[hf] = _pk(fm[hf])
        g_s[hf] = _pk(gm[hf])
    bk_s[:, 0:PADK, :] = jnp.zeros((NCG, PADK, 128), BF16)

    for cp in cp_small:
        cp.start()
    start_kvaux(0, 0)
    cp_c(1).start()
    start_kvaux(0, 1)

    for b in range(4):
        cp_wuk(0, b).wait()
        cp_wuv(0, b).wait()
        for s in range(4):
            relayout_wkv_step(0, b, s, 0)
            relayout_wkv_step(0, b, s, 1)

    for b in range(2, 4):
        cp_c(b).start()
        start_kvaux(0, b)
    for b in range(4):
        cp_x(b).start()
    cp_h(0).start()
    cp_h(1).start()
    for cp in cp_small:
        cp.wait()
    cp_c(0).wait()
    for rb in range(RC // 128):
        stage_c(0, rb)

    def group_body(g, carry):
        @pl.when(g + 1 < NG)
        def _():
            start_wkv(g + 1)
            for b in range(4):
                start_kvaux(g + 1, b)
            cp_h(2 * g + 2).start()
            cp_h(2 * g + 3).start()

        @pl.when(g == 1)
        def _():
            cp_wo.start()

        def kv_body(b, c2):
            p = g * 4 + b

            def waits():
                @pl.when(jnp.logical_and(g == 0, b + 1 < NRC))
                def _():
                    cp_c(b + 1).wait()
                cp_wq(g, b).wait()
                cp_bk(p).wait()
                cp_bv(p).wait()
            _own_block(jnp.minimum(b + 1, 1), waits)
            bn = (b + 1) % NRC

            def mm_piece(rb, hh):
                def run():
                    prow = pl.ds(pl.multiple_of(b * (RC // 2) + rb * 64, 64), 64)
                    kk = jnp.dot(_up(c_p[rb * 64:(rb + 1) * 64, :]), _up(wkv_s[:, hh * 256:(hh + 1) * 256]),
                                 preferred_element_type=F32)
                    k_s[hh, prow, :] = _pk(kk[:, 0:128].astype(BF16))
                    v_s[hh, prow, :] = _pk(kk[:, 128:256].astype(BF16))
                return run

            def rq_step(s):
                def run():
                    m0 = pl.multiple_of(b * 256 + s * 32, 32)
                    t = jnp.swapaxes(wq_raw[g, pl.ds(m0, 32)], 0, 1)
                    prow = pl.ds(pl.multiple_of(b * 128 + s * 16, 16), 16)
                    for hh in range(HG):
                        wq_s[prow, hh * 128:(hh + 1) * 128] = _pk(t[hh])
                return run

            cg = p // 2
            rh = p % 2
            w = sk_v[:, pl.ds(pl.multiple_of(cg * 128, 128), 128)].astype(F32)

            def kvb_step(s):
                def run():
                    r0 = pl.multiple_of(rh * 1024 + s * 64, 64)
                    kw = bk_s[cg, pl.ds(r0, 64 + PADK), :].astype(F32)
                    acc = kw[PADK:] * w[0:1]
                    for j in range(1, 4):
                        acc = acc + kw[PADK - j:PADK - j + 64] * w[j:j + 1]
                    kvv = acc * bv_s[cg, pl.ds(r0, 64), :].astype(F32)
                    kv_s[cg, pl.ds(pl.multiple_of(rh * 512 + s * 32, 32), 32), :] = _pk(kvv.astype(BF16))
                return run

            aux = []
            for s in range(8):
                aux += [rq_step(s), kvb_step(2 * s), kvb_step(2 * s + 1)]
            k = 0
            done = 0
            for rb in range(RC // 128):
                for hh in range(HG):
                    mm_piece(rb, hh)()
                    k += 1
                    tgt = min(len(aux), (len(aux) * k) // 30)
                    while done < tgt:
                        aux[done]()
                        done += 1
                stage_c(bn, rb)
            return c2

        lax.fori_loop(0, NRC, kv_body, 0)

        def q_body(b, c2):
            bn = (b + 1) % NRC
            p = g * 4 + b
            cg = p // 2
            hf = p % 2

            def waits():
                @pl.when(jnp.logical_and(g == 0, b + 1 < NRC))
                def _():
                    cp_x(b + 1).wait()

                @pl.when(hf == 0)
                def _():
                    cp_h(cg).wait()

                @pl.when(g + 1 < NG)
                def _():
                    cp_wuk(g + 1, b).wait()
                    cp_wuv(g + 1, b).wait()
            _own_block(jnp.minimum(b + 1, 1), waits)

            gn = jnp.minimum(g + 1, NG - 1)
            fh = _up(f_s[hf])
            gh = _up(g_s[hf])
            st = {}

            def q_piece(rb, hh):
                def run():
                    prow = pl.ds(pl.multiple_of(b * (RC // 2) + rb * 64, 64), 64)
                    qq = jnp.dot(_up(x_p[rb * 64:(rb + 1) * 64, :]), _up(wq_s[:, hh * 128:(hh + 1) * 128]),
                                 preferred_element_type=F32) * QSCALE
                    q_s[hh, prow, :] = _pk(qq.astype(BF16))
                return run

            def u_piece(q):
                def run():
                    ucat = jnp.concatenate(
                        [_up(kv_s[cg, i * 64:(i + 1) * 64, :]) for i in range(4 * q, 4 * q + 4)], axis=1)
                    u_s[:, q * 512:(q + 1) * 512] = jnp.dot(fh, ucat, preferred_element_type=F32)
                return run

            def h_piece(q):
                def run():
                    hcat = jnp.concatenate(
                        [h_s[cg, :, m * CB:(m + 1) * CB] for m in range(4 * q, 4 * q + 4)], axis=0)
                    st["hh", q] = lax.dot_general(fh, hcat, NT, preferred_element_type=F32)
                return run

            sgn = jnp.where((lax.broadcasted_iota(jnp.int32, (64, 128), 0) & 1) == 0,
                            1.0, -1.0).astype(F32)

            def t_step(m):
                def run():
                    cur = st["hh", m // 4][:, (m % 4) * CB:(m % 4 + 1) * CB]
                    tr = sgn * cur[64:128]
                    ti = sgn * cur[0:64]
                    if m > 0:
                        prv = st["hh", (m - 1) // 4][:, ((m - 1) % 4) * CB:((m - 1) % 4 + 1) * CB]
                        tr = prv[0:64] + tr
                        ti = prv[64:128] - ti
                    else:
                        ti = -ti
                    ht_s[0:64, m * CB:(m + 1) * CB] = tr
                    ht_s[64:128, m * CB:(m + 1) * CB] = ti
                return run

            RB = 32

            def p_step(i, rb, m):
                def run():
                    a0 = (i - m) * CB
                    b0 = m * CB
                    ur = u_s[rb:rb + RB, a0:a0 + CB]
                    ui = u_s[64 + rb:64 + rb + RB, a0:a0 + CB]
                    hr = ht_s[rb:rb + RB, b0:b0 + CB]
                    hi = ht_s[64 + rb:64 + rb + RB, b0:b0 + CB]
                    pr = ur * hr - ui * hi
                    pi = ur * hi + ui * hr
                    if m > 0:
                        pr = st["yr"] + pr
                        pi = st["yi"] + pi
                    st["yr"], st["yi"] = pr, pi
                    if m == i:
                        st["Y", i, rb] = (pr.astype(BF16), pi.astype(BF16))
                return run

            def i_piece(q):
                def run():
                    blocks = []
                    for i in range(4 * q, 4 * q + 4):
                        parts = [st.pop(("Y", i, rb)) for rb in range(0, 64, RB)]
                        blocks.append(jnp.concatenate([t[0] for t in parts] + [t[1] for t in parts], axis=0))
                    st["yo", q] = jnp.dot(gh, jnp.concatenate(blocks, axis=1), preferred_element_type=F32)
                return run

            def y_step(i):
                def run():
                    yo = st["yo", i // 4][:, (i % 4) * CB:(i % 4 + 1) * CB]
                    old = jnp.where(hf == 0, 0.0, y_s[cg, i * CB:(i + 1) * CB, :])
                    y_s[cg, i * CB:(i + 1) * CB, :] = old + yo
                return run

            rsteps = [(lambda s=s, wh=wh: relayout_wkv_step(gn, b, s, wh)) for s in range(4) for wh in range(2)]
            for q in range(4):
                u_piece(q)()
            for q in range(4):
                h_piece(q)()
            qp = [q_piece(rb, hh) for rb in range(RC // 128) for hh in range(HG)]
            aux = [t_step(m) for m in range(NCB)]
            psteps = [(i, rb, m) for i in range(NCB) for rb in range(0, 64, RB) for m in range(i + 1)]
            NQ1 = 28
            per = len(psteps) / float(NQ1 - 1)
            done = 0
            pend_i = [0, 1, 2, 3]
            pend_y = []
            for k in range(len(qp)):
                qp[k]()
                if k % HG == HG - 1:
                    stage_x(bn, k // HG)
                if k == 0:
                    for a in aux:
                        a()
                    continue
                while pend_i and done >= 2 * sum(range(1, 4 * pend_i[0] + 5)):
                    q = pend_i.pop(0)
                    i_piece(q)()
                    pend_y += list(range(4 * q, 4 * q + 4))
                    break
                tgt = min(len(psteps), int(round(per * k)))
                while done < tgt:
                    p_step(*psteps[done])()
                    done += 1
                if k % 3 == 2 and rsteps:
                    rsteps.pop(0)()
                ny = 1 if pend_i else 2
                for _ in range(ny):
                    if pend_y:
                        y_step(pend_y.pop(0))()
            assert not pend_i and not rsteps
            while pend_y:
                y_step(pend_y.pop(0))()
            return c2

        @pl.when(g == 0)
        def _():
            cp_x(0).wait()
            for rb in range(RC // 128):
                stage_x(0, rb)

        lax.fori_loop(0, NRC, q_body, 0)

        mask = (lax.broadcasted_iota(jnp.int32, (BQ, BQ), 1)
                <= lax.broadcasted_iota(jnp.int32, (BQ, BQ), 0))
        HB = BQ // 2

        def attn_body(t, c2):
            def qk(hh, i):
                return lax.dot_general(_up(q_s[hh, i * HB:(i + 1) * HB, :]),
                                       _up(k_s[hh, 0:(i + 1) * HB, :]), NT,
                                       preferred_element_type=F32)

            def sm(i, s):
                L = (i + 1) * BQ
                sd = jnp.where(mask, s[:, L - BQ:], NEG)
                s = jnp.concatenate([s[:, :L - BQ], sd], axis=1) if i > 0 else sd
                m = jnp.max(s, axis=1, keepdims=True)
                p = jnp.exp2(s - m)
                l = jnp.sum(p, axis=1, keepdims=True)
                return p.astype(BF16), l

            def pv(hh, i, p, l):
                ctx = jnp.dot(p, _up(v_s[hh, 0:(i + 1) * HB, :]), preferred_element_type=F32)
                r = pl.reciprocal(l, approx=True)
                r = r * (2.0 - l * r)
                ctx_s[g * HG + hh, i * HB:(i + 1) * HB, :] = _pk((ctx * r).astype(BF16))

            order = [(2 * t + u, i) for i in range(NBQ)[::-1] for u in range(2)]
            s_next = qk(*order[0])
            for n, (hh, i) in enumerate(order):
                s = s_next
                if n + 1 < len(order):
                    s_next = qk(*order[n + 1])
                p, l = sm(i, s)
                pv(hh, i, p, l)
            return c2

        lax.fori_loop(0, HG // 2, attn_body, 0)
        return carry

    lax.fori_loop(0, NG, group_body, 0)

    cp_wo.wait()

    def out_body(r, carry):
        rows = pl.ds(pl.multiple_of(r * FO, FO), FO)
        prow = pl.ds(pl.multiple_of(r * (FO // 2), FO // 2), FO // 2)
        ctx = jnp.concatenate([_up(ctx_s[hh, prow, :]) for hh in range(H)], axis=1)
        a = jnp.dot(ctx, wo_v[...], preferred_element_type=F32)
        xf = x_v[rows, :].astype(F32)
        gw = gw_v[...].astype(F32)[None, :]
        gate = jax.nn.sigmoid(jnp.sum(xf * gw, axis=1, keepdims=True))
        dd = d_v[...].astype(F32)[None, :]
        for cg in range(NCG):
            cols = slice(cg * 128, (cg + 1) * 128)
            yb = y_s[cg, rows, :] + _up(kv_s[cg, prow, :]).astype(F32) * dd[:, cols]
            o_s[rows, cols] = (gate * a[:, cols] + (1.0 - gate) * (xf[:, cols] * yb)).astype(BF16)
        cp_o(r).start()
        return carry

    lax.fori_loop(0, S // FO, out_body, 0)
    for r in range(S // FO):
        cp_o(r).wait()


@jax.jit
def pallas_gated_mix__compressed_kv_cla__ssm_conv_h3__prompt_kernel(
    A_x: jax.Array,
    A_c_kv: jax.Array,
    A_w_q: jax.Array,
    A_w_uk: jax.Array,
    A_w_uv: jax.Array,
    A_w_o: jax.Array,
    B_q: jax.Array,
    B_k: jax.Array,
    B_v: jax.Array,
    B_shift_k: jax.Array,
    B_ssm_k: jax.Array,
    B_ssm_D: jax.Array,
    gate_w: jax.Array,
):
    del B_q
    x = A_x.reshape(S, M)
    c = A_c_kv.reshape(S, DC)
    wq = A_w_q.reshape(M, NG, HG, D)
    wuk = A_w_uk.reshape(DC, NG, HG, D)
    wuv = A_w_uv.reshape(DC, NG, HG, D)
    wo = A_w_o.reshape(H * D, M)
    bk = B_k.reshape(S, M)
    bv = B_v.reshape(S, M)
    skt = B_shift_k.T

    dma = pltpu.SemaphoreType.DMA
    scratch = [
        pltpu.VMEM((S, M), BF16),
        pltpu.VMEM((S, DC), BF16),
        pltpu.VMEM((NG, M, HG, D), BF16),
        pltpu.VMEM((NG, DC, HG, D), BF16),
        pltpu.VMEM((NG, DC, HG, D), BF16),
        pltpu.VMEM((H * D, M), BF16),
        pltpu.VMEM((NCG, PADK + S, 128), BF16),
        pltpu.VMEM((NCG, S, 128), BF16),
        pltpu.VMEM((NCG, 128, S), BF16),
        pltpu.VMEM((RC // 2, M), U32),
        pltpu.VMEM((RC // 2, DC), U32),
        pltpu.VMEM((M // 2, HG * D), U32),
        pltpu.VMEM((DC // 2, 2 * HG * D), U32),
        pltpu.VMEM((HG, S // 2, D), U32),
        pltpu.VMEM((HG, S // 2, D), U32),
        pltpu.VMEM((HG, S // 2, D), U32),
        pltpu.VMEM((H, S // 2, D), U32),
        pltpu.VMEM((NCG, S // 2, 128), U32),
        pltpu.VMEM((NCG, S, 128), F32),
        pltpu.VMEM((128, S), F32),
        pltpu.VMEM((128, S), F32),
        pltpu.VMEM((2, 64, 128), U32),
        pltpu.VMEM((2, 64, 128), U32),
        pltpu.VMEM((S, M), BF16),
        pltpu.VMEM((4, M), BF16),
        pltpu.VMEM((M,), BF16),
        pltpu.VMEM((M,), BF16),
        dma((4,)), dma((4,)), dma((16,)), dma((16,)), dma((16,)), dma((1,)),
        dma((16,)), dma((16,)), dma((8,)), dma((3,)), dma((S // FO,)),
    ]
    out = pl.pallas_call(
        _kernel,
        out_shape=jax.ShapeDtypeStruct((S, M), BF16),
        in_specs=[pl.BlockSpec(memory_space=pl.ANY)] * 12,
        out_specs=pl.BlockSpec(memory_space=pl.ANY),
        scratch_shapes=scratch,
        compiler_params=pltpu.CompilerParams(vmem_limit_bytes=120 * 1024 * 1024),
    )(x, c, wq, wuk, wuv, wo, bk, bv, skt, B_ssm_k, B_ssm_D, gate_w)
    return out.reshape(1, S, M)
```

```python
import math

import jax
import jax.numpy as jnp
from jax import lax
import jax.experimental.pallas as pl
import jax.experimental.pallas.tpu as pltpu

F32 = jnp.float32
BF16 = jnp.bfloat16

S = 2048
M = 1024
H = 32
D = 128
DC = 512
HG = 8
NG = H // HG
RC = 512
NRC = S // RC
BQ = 128
NBQ = S // BQ
CB = 128
NCB = S // CB
NCG = M // 128
FO = 256
PADK = 16
NEG = -1e9
NT = (((1,), (1,)), ((), ()))
QSCALE = (D ** -0.5) * math.log2(math.e)


def _dft_mats():
    shp = (2, 128, 128)
    hf = lax.broadcasted_iota(jnp.int32, shp, 0)
    r = lax.broadcasted_iota(jnp.int32, shp, 1)
    j = lax.broadcasted_iota(jnp.int32, shp, 2)
    f = hf * 64 + (r & 63)
    k = ((2 * f + 1) * j + jnp.where(r >= 64, 128, 0)) & 511
    fm = jnp.cos(k.astype(F32) * (2 * math.pi / 512))
    ff = hf * 64 + (j & 63)
    k2 = ((2 * ff + 1) * (r + 128) + jnp.where(j >= 64, 128, 0)) & 511
    gm = jnp.cos(k2.astype(F32) * (2 * math.pi / 512)) * (1.0 / 128)
    return fm.astype(BF16), gm.astype(BF16)


U32 = jnp.uint32


def _pk(v):
    return pltpu.bitcast(v, U32)


def _up(v):
    return pltpu.bitcast(v, BF16)


def _own_block(trips, fn):
    def body(_, c):
        fn()
        return c
    lax.fori_loop(0, trips, body, 0)


def _spread(pieces, aux):
    n = len(pieces)
    done = 0
    for k, piece in enumerate(pieces):
        piece()
        tgt = (len(aux) * (k + 1)) // n
        while done < tgt:
            aux[done]()
            done += 1


def _kernel(x_h, c_h, wq_h, wuk_h, wuv_h, wo_h, bk_h, bv_h, sk_h, h_h, d_h, gw_h,
            o_h,
            x_v, c_v, wq_raw, wuk_raw, wuv_raw, wo_v, bk_s, bv_s, h_s,
            x_p, c_p, wq_s, wkv_s, q_s, k_s, v_s, ctx_s, kv_s, y_s, u_s, ht_s, f_s, g_s, o_s,
            sk_v, d_v, gw_v,
            sem_c, sem_x, sem_wq, sem_wuk, sem_wuv, sem_wo, sem_bk, sem_bv,
            sem_h, sem_small, sem_o):
    def cp_c(b):
        return pltpu.make_async_copy(c_h.at[pl.ds(b * RC, RC)], c_v.at[pl.ds(b * RC, RC)], sem_c.at[b])

    def cp_x(b):
        return pltpu.make_async_copy(x_h.at[pl.ds(b * RC, RC)], x_v.at[pl.ds(b * RC, RC)], sem_x.at[b])

    def cp_wq(g, b):
        rows = pl.ds(b * 256, 256)
        return pltpu.make_async_copy(wq_h.at[rows, g], wq_raw.at[g, rows], sem_wq.at[g * 4 + b])

    def cp_wuk(g, b):
        rows = pl.ds(b * 128, 128)
        return pltpu.make_async_copy(wuk_h.at[rows, g], wuk_raw.at[g, rows], sem_wuk.at[g * 4 + b])

    def cp_wuv(g, b):
        rows = pl.ds(b * 128, 128)
        return pltpu.make_async_copy(wuv_h.at[rows, g], wuv_raw.at[g, rows], sem_wuv.at[g * 4 + b])

    def cp_bk(p):
        cg = p // 2
        r0 = (p % 2) * 1024
        return pltpu.make_async_copy(bk_h.at[pl.ds(r0, 1024), pl.ds(cg * 128, 128)],
                                     bk_s.at[cg, pl.ds(PADK + r0, 1024)], sem_bk.at[p])

    def cp_bv(p):
        cg = p // 2
        rows = pl.ds((p % 2) * 1024, 1024)
        return pltpu.make_async_copy(bv_h.at[rows, pl.ds(cg * 128, 128)], bv_s.at[cg, rows], sem_bv.at[p])

    def cp_h(cg):
        return pltpu.make_async_copy(h_h.at[pl.ds(cg * 128, 128)], h_s.at[cg], sem_h.at[cg])

    cp_wo = pltpu.make_async_copy(wo_h, wo_v, sem_wo.at[0])
    cp_small = [pltpu.make_async_copy(sk_h, sk_v, sem_small.at[0]),
                pltpu.make_async_copy(d_h, d_v, sem_small.at[1]),
                pltpu.make_async_copy(gw_h, gw_v, sem_small.at[2])]

    def cp_o(r):
        rows = pl.ds(r * FO, FO)
        return pltpu.make_async_copy(o_s.at[rows], o_h.at[rows], sem_o.at[r])

    def start_kvaux(g, b):
        cp_wq(g, b).start()
        cp_bk(g * 4 + b).start()
        cp_bv(g * 4 + b).start()

    def start_wkv(g):
        for b in range(4):
            cp_wuk(g, b).start()
            cp_wuv(g, b).start()

    def relayout_wkv_step(g, b, s, which):
        m0 = pl.multiple_of(b * 128 + s * 32, 32)
        src = wuk_raw if which == 0 else wuv_raw
        t = jnp.swapaxes(src[g, pl.ds(m0, 32)], 0, 1)
        prow = pl.ds(pl.multiple_of(b * 64 + s * 16, 16), 16)
        for hh in range(HG):
            c0 = hh * 256 + which * 128
            wkv_s[prow, c0:c0 + 128] = _pk(t[hh])

    def stage_c(bn, rb):
        c_p[rb * 64:(rb + 1) * 64, :] = _pk(c_v[pl.ds(pl.multiple_of(bn * RC + rb * 128, 128), 128), :])

    def stage_x(bn, rb):
        x_p[rb * 64:(rb + 1) * 64, :] = _pk(x_v[pl.ds(pl.multiple_of(bn * RC + rb * 128, 128), 128), :])

    start_wkv(0)
    cp_c(0).start()

    fm, gm = _dft_mats()
    for hf in range(2):
        f_s[hf] = _pk(fm[hf])
        g_s[hf] = _pk(gm[hf])
    bk_s[:, 0:PADK, :] = jnp.zeros((NCG, PADK, 128), BF16)

    for cp in cp_small:
        cp.start()
    start_kvaux(0, 0)
    cp_c(1).start()
    start_kvaux(0, 1)

    for b in range(4):
        cp_wuk(0, b).wait()
        cp_wuv(0, b).wait()
        for s in range(4):
            relayout_wkv_step(0, b, s, 0)
            relayout_wkv_step(0, b, s, 1)

    for b in range(2, 4):
        cp_c(b).start()
        start_kvaux(0, b)
    for b in range(4):
        cp_x(b).start()
    cp_h(0).start()
    cp_h(1).start()
    for cp in cp_small:
        cp.wait()
    cp_c(0).wait()
    for rb in range(RC // 128):
        stage_c(0, rb)

    def group_body(g, carry):
        @pl.when(g + 1 < NG)
        def _():
            start_wkv(g + 1)
            for b in range(4):
                start_kvaux(g + 1, b)
            cp_h(2 * g + 2).start()
            cp_h(2 * g + 3).start()

        @pl.when(g == 1)
        def _():
            cp_wo.start()

        def kv_body(b, c2):
            p = g * 4 + b

            def waits():
                @pl.when(jnp.logical_and(g == 0, b + 1 < NRC))
                def _():
                    cp_c(b + 1).wait()
                cp_wq(g, b).wait()
                cp_bk(p).wait()
                cp_bv(p).wait()
            _own_block(jnp.minimum(b + 1, 1), waits)
            bn = (b + 1) % NRC

            def mm_piece(rb, hh):
                def run():
                    prow = pl.ds(pl.multiple_of(b * (RC // 2) + rb * 64, 64), 64)
                    kk = jnp.dot(_up(c_p[rb * 64:(rb + 1) * 64, :]), _up(wkv_s[:, hh * 256:(hh + 1) * 256]),
                                 preferred_element_type=F32)
                    k_s[hh, prow, :] = _pk(kk[:, 0:128].astype(BF16))
                    v_s[hh, prow, :] = _pk(kk[:, 128:256].astype(BF16))
                return run

            def rq_step(s):
                def run():
                    m0 = pl.multiple_of(b * 256 + s * 32, 32)
                    t = jnp.swapaxes(wq_raw[g, pl.ds(m0, 32)], 0, 1)
                    prow = pl.ds(pl.multiple_of(b * 128 + s * 16, 16), 16)
                    for hh in range(HG):
                        wq_s[prow, hh * 128:(hh + 1) * 128] = _pk(t[hh])
                return run

            cg = p // 2
            rh = p % 2
            w = sk_v[:, pl.ds(pl.multiple_of(cg * 128, 128), 128)].astype(F32)

            def kvb_step(s):
                def run():
                    r0 = pl.multiple_of(rh * 1024 + s * 64, 64)
                    kw = bk_s[cg, pl.ds(r0, 64 + PADK), :].astype(F32)
                    acc = kw[PADK:] * w[0:1]
                    for j in range(1, 4):
                        acc = acc + kw[PADK - j:PADK - j + 64] * w[j:j + 1]
                    kvv = acc * bv_s[cg, pl.ds(r0, 64), :].astype(F32)
                    kv_s[cg, pl.ds(pl.multiple_of(rh * 512 + s * 32, 32), 32), :] = _pk(kvv.astype(BF16))
                return run

            aux = []
            for s in range(8):
                aux += [rq_step(s), kvb_step(2 * s), kvb_step(2 * s + 1)]
            k = 0
            done = 0
            for rb in range(RC // 128):
                for hh in range(HG):
                    mm_piece(rb, hh)()
                    k += 1
                    tgt = min(len(aux), (len(aux) * k) // 30)
                    while done < tgt:
                        aux[done]()
                        done += 1
                stage_c(bn, rb)
            return c2

        lax.fori_loop(0, NRC, kv_body, 0)

        def q_body(b, c2):
            bn = (b + 1) % NRC
            p = g * 4 + b
            cg = p // 2
            hf = p % 2

            def waits():
                @pl.when(jnp.logical_and(g == 0, b + 1 < NRC))
                def _():
                    cp_x(b + 1).wait()

                @pl.when(hf == 0)
                def _():
                    cp_h(cg).wait()

                @pl.when(g + 1 < NG)
                def _():
                    cp_wuk(g + 1, b).wait()
                    cp_wuv(g + 1, b).wait()
            _own_block(jnp.minimum(b + 1, 1), waits)

            gn = jnp.minimum(g + 1, NG - 1)
            fh = _up(f_s[hf])
            gh = _up(g_s[hf])
            st = {}

            def q_piece(rb, hh):
                def run():
                    prow = pl.ds(pl.multiple_of(b * (RC // 2) + rb * 64, 64), 64)
                    qq = jnp.dot(_up(x_p[rb * 64:(rb + 1) * 64, :]), _up(wq_s[:, hh * 128:(hh + 1) * 128]),
                                 preferred_element_type=F32) * QSCALE
                    q_s[hh, prow, :] = _pk(qq.astype(BF16))
                return run

            def u_piece(q):
                def run():
                    ucat = jnp.concatenate(
                        [_up(kv_s[cg, i * 64:(i + 1) * 64, :]) for i in range(4 * q, 4 * q + 4)], axis=1)
                    u_s[:, q * 512:(q + 1) * 512] = jnp.dot(fh, ucat, preferred_element_type=F32)
                return run

            def h_piece(q):
                def run():
                    hcat = jnp.concatenate(
                        [h_s[cg, :, m * CB:(m + 1) * CB] for m in range(4 * q, 4 * q + 4)], axis=0)
                    st["hh", q] = lax.dot_general(fh, hcat, NT, preferred_element_type=F32)
                return run

            sgn = jnp.where((lax.broadcasted_iota(jnp.int32, (64, 128), 0) & 1) == 0,
                            1.0, -1.0).astype(F32)

            def t_step(m):
                def run():
                    cur = st["hh", m // 4][:, (m % 4) * CB:(m % 4 + 1) * CB]
                    tr = sgn * cur[64:128]
                    ti = sgn * cur[0:64]
                    if m > 0:
                        prv = st["hh", (m - 1) // 4][:, ((m - 1) % 4) * CB:((m - 1) % 4 + 1) * CB]
                        tr = prv[0:64] + tr
                        ti = prv[64:128] - ti
                    else:
                        ti = -ti
                    ht_s[0:64, m * CB:(m + 1) * CB] = tr
                    ht_s[64:128, m * CB:(m + 1) * CB] = ti
                return run

            RB = 32

            def p_step(i, rb, m):
                def run():
                    a0 = (i - m) * CB
                    b0 = m * CB
                    ur = u_s[rb:rb + RB, a0:a0 + CB]
                    ui = u_s[64 + rb:64 + rb + RB, a0:a0 + CB]
                    hr = ht_s[rb:rb + RB, b0:b0 + CB]
                    hi = ht_s[64 + rb:64 + rb + RB, b0:b0 + CB]
                    pr = ur * hr - ui * hi
                    pi = ur * hi + ui * hr
                    if m > 0:
                        pr = st["yr"] + pr
                        pi = st["yi"] + pi
                    st["yr"], st["yi"] = pr, pi
                    if m == i:
                        st["Y", i, rb] = (pr.astype(BF16), pi.astype(BF16))
                return run

            def i_piece(q):
                def run():
                    blocks = []
                    for i in range(4 * q, 4 * q + 4):
                        parts = [st.pop(("Y", i, rb)) for rb in range(0, 64, RB)]
                        blocks.append(jnp.concatenate([t[0] for t in parts] + [t[1] for t in parts], axis=0))
                    st["yo", q] = jnp.dot(gh, jnp.concatenate(blocks, axis=1), preferred_element_type=F32)
                return run

            def y_step(i):
                def run():
                    yo = st["yo", i // 4][:, (i % 4) * CB:(i % 4 + 1) * CB]
                    old = jnp.where(hf == 0, 0.0, y_s[cg, i * CB:(i + 1) * CB, :])
                    y_s[cg, i * CB:(i + 1) * CB, :] = old + yo
                return run

            rsteps = [(lambda s=s, wh=wh: relayout_wkv_step(gn, b, s, wh)) for s in range(4) for wh in range(2)]
            for q in range(4):
                u_piece(q)()
            for q in range(4):
                h_piece(q)()
            qp = [q_piece(rb, hh) for rb in range(RC // 128) for hh in range(HG)]
            aux = [t_step(m) for m in range(NCB)]
            psteps = [(i, rb, m) for i in range(NCB) for rb in range(0, 64, RB) for m in range(i + 1)]
            NQ1 = 28
            per = len(psteps) / float(NQ1 - 1)
            done = 0
            pend_i = [0, 1, 2, 3]
            pend_y = []
            for k in range(len(qp)):
                qp[k]()
                if k % HG == HG - 1:
                    stage_x(bn, k // HG)
                if k == 0:
                    for a in aux:
                        a()
                    continue
                while pend_i and done >= 2 * sum(range(1, 4 * pend_i[0] + 5)):
                    q = pend_i.pop(0)
                    i_piece(q)()
                    pend_y += list(range(4 * q, 4 * q + 4))
                    break
                tgt = min(len(psteps), int(round(per * k)))
                while done < tgt:
                    p_step(*psteps[done])()
                    done += 1
                if k % 3 == 2 and rsteps:
                    rsteps.pop(0)()
                ny = 1 if pend_i else 2
                for _ in range(ny):
                    if pend_y:
                        y_step(pend_y.pop(0))()
            assert not pend_i and not rsteps
            while pend_y:
                y_step(pend_y.pop(0))()
            return c2

        @pl.when(g == 0)
        def _():
            cp_x(0).wait()
            for rb in range(RC // 128):
                stage_x(0, rb)

        lax.fori_loop(0, NRC, q_body, 0)

        mask = (lax.broadcasted_iota(jnp.int32, (BQ, BQ), 1)
                <= lax.broadcasted_iota(jnp.int32, (BQ, BQ), 0))
        HB = BQ // 2

        def attn_body(t, c2):
            def qk(hh, i, z):
                q = q_s[hh, i * HB:(i + 1) * HB, :]
                if z is not None:
                    q = jnp.concatenate([q[0:8] + z, q[8:]], axis=0)
                return lax.dot_general(_up(q), _up(k_s[hh, 0:(i + 1) * HB, :]), NT,
                                       preferred_element_type=F32)

            def sm(i, s):
                L = (i + 1) * BQ
                sd = jnp.where(mask, s[:, L - BQ:], NEG)
                s = jnp.concatenate([s[:, :L - BQ], sd], axis=1) if i > 0 else sd
                m = jnp.max(s, axis=1, keepdims=True)
                p = jnp.exp2(s - m)
                l = jnp.sum(p, axis=1, keepdims=True)
                return p.astype(BF16), l

            def pv(hh, i, p):
                return jnp.dot(p, _up(v_s[hh, 0:(i + 1) * HB, :]), preferred_element_type=F32)

            def fin(hh, i, ctx, l):
                r = pl.reciprocal(l, approx=True)
                r = r * (2.0 - l * r)
                o = _pk((ctx * r).astype(BF16))
                ctx_s[g * HG + hh, i * HB:(i + 1) * HB, :] = o
                a = o[0:8]
                for kk in range(1, 8):
                    a = a | o[8 * kk:8 * kk + 8]
                return (a & 1) >> 1

            ha, hb = 2 * t, 2 * t + 1
            order = []
            for i in range(NBQ // 2):
                order += [(ha, NBQ - 1 - i), (hb, NBQ - 1 - i), (hb, i), (ha, i)]
            n = len(order)
            lag = 3
            ss, cs, zs = {}, {}, {}
            ss[0] = qk(*order[0], None)
            for j in range(n + lag):
                if j + 1 < n:
                    ss[j + 1] = qk(*order[j + 1], zs.pop(j + 1, None))
                if j < n:
                    p, l = sm(order[j][1], ss.pop(j))
                    cs[j] = (pv(*order[j], p), l)
                if 0 <= j - lag < n:
                    zs[j + 2] = fin(*order[j - lag], *cs.pop(j - lag))
            return c2

        lax.fori_loop(0, HG // 2, attn_body, 0)
        return carry

    lax.fori_loop(0, NG, group_body, 0)

    cp_wo.wait()

    def out_body(r, carry):
        rows = pl.ds(pl.multiple_of(r * FO, FO), FO)
        prow = pl.ds(pl.multiple_of(r * (FO // 2), FO // 2), FO // 2)
        ctx = jnp.concatenate([_up(ctx_s[hh, prow, :]) for hh in range(H)], axis=1)
        a = jnp.dot(ctx, wo_v[...], preferred_element_type=F32)
        xf = x_v[rows, :].astype(F32)
        gw = gw_v[...].astype(F32)[None, :]
        gate = jax.nn.sigmoid(jnp.sum(xf * gw, axis=1, keepdims=True))
        dd = d_v[...].astype(F32)[None, :]
        for cg in range(NCG):
            cols = slice(cg * 128, (cg + 1) * 128)
            yb = y_s[cg, rows, :] + _up(kv_s[cg, prow, :]).astype(F32) * dd[:, cols]
            o_s[rows, cols] = (gate * a[:, cols] + (1.0 - gate) * (xf[:, cols] * yb)).astype(BF16)
        cp_o(r).start()
        return carry

    lax.fori_loop(0, S // FO, out_body, 0)
    for r in range(S // FO):
        cp_o(r).wait()


@jax.jit
def pallas_gated_mix__compressed_kv_cla__ssm_conv_h3__prompt_kernel(
    A_x: jax.Array,
    A_c_kv: jax.Array,
    A_w_q: jax.Array,
    A_w_uk: jax.Array,
    A_w_uv: jax.Array,
    A_w_o: jax.Array,
    B_q: jax.Array,
    B_k: jax.Array,
    B_v: jax.Array,
    B_shift_k: jax.Array,
    B_ssm_k: jax.Array,
    B_ssm_D: jax.Array,
    gate_w: jax.Array,
):
    del B_q
    x = A_x.reshape(S, M)
    c = A_c_kv.reshape(S, DC)
    wq = A_w_q.reshape(M, NG, HG, D)
    wuk = A_w_uk.reshape(DC, NG, HG, D)
    wuv = A_w_uv.reshape(DC, NG, HG, D)
    wo = A_w_o.reshape(H * D, M)
    bk = B_k.reshape(S, M)
    bv = B_v.reshape(S, M)
    skt = B_shift_k.T

    dma = pltpu.SemaphoreType.DMA
    scratch = [
        pltpu.VMEM((S, M), BF16),
        pltpu.VMEM((S, DC), BF16),
        pltpu.VMEM((NG, M, HG, D), BF16),
        pltpu.VMEM((NG, DC, HG, D), BF16),
        pltpu.VMEM((NG, DC, HG, D), BF16),
        pltpu.VMEM((H * D, M), BF16),
        pltpu.VMEM((NCG, PADK + S, 128), BF16),
        pltpu.VMEM((NCG, S, 128), BF16),
        pltpu.VMEM((NCG, 128, S), BF16),
        pltpu.VMEM((RC // 2, M), U32),
        pltpu.VMEM((RC // 2, DC), U32),
        pltpu.VMEM((M // 2, HG * D), U32),
        pltpu.VMEM((DC // 2, 2 * HG * D), U32),
        pltpu.VMEM((HG, S // 2, D), U32),
        pltpu.VMEM((HG, S // 2, D), U32),
        pltpu.VMEM((HG, S // 2, D), U32),
        pltpu.VMEM((H, S // 2, D), U32),
        pltpu.VMEM((NCG, S // 2, 128), U32),
        pltpu.VMEM((NCG, S, 128), F32),
        pltpu.VMEM((128, S), F32),
        pltpu.VMEM((128, S), F32),
        pltpu.VMEM((2, 64, 128), U32),
        pltpu.VMEM((2, 64, 128), U32),
        pltpu.VMEM((S, M), BF16),
        pltpu.VMEM((4, M), BF16),
        pltpu.VMEM((M,), BF16),
        pltpu.VMEM((M,), BF16),
        dma((4,)), dma((4,)), dma((16,)), dma((16,)), dma((16,)), dma((1,)),
        dma((16,)), dma((16,)), dma((8,)), dma((3,)), dma((S // FO,)),
    ]
    out = pl.pallas_call(
        _kernel,
        out_shape=jax.ShapeDtypeStruct((S, M), BF16),
        in_specs=[pl.BlockSpec(memory_space=pl.ANY)] * 12,
        out_specs=pl.BlockSpec(memory_space=pl.ANY),
        scratch_shapes=scratch,
        compiler_params=pltpu.CompilerParams(vmem_limit_bytes=120 * 1024 * 1024),
    )(x, c, wq, wuk, wuv, wo, bk, bv, skt, B_ssm_k, B_ssm_D, gate_w)
    return out.reshape(1, S, M)
```

```python
import math

import jax
import jax.numpy as jnp
from jax import lax
import jax.experimental.pallas as pl
import jax.experimental.pallas.tpu as pltpu

F32 = jnp.float32
BF16 = jnp.bfloat16

S = 2048
M = 1024
H = 32
D = 128
DC = 512
HG = 8
NG = H // HG
RC = 512
NRC = S // RC
BQ = 128
NBQ = S // BQ
AH = 2
CB = 128
NCB = S // CB
NCG = M // 128
FO = 256
PADK = 16
NEG = -1e9
NT = (((1,), (1,)), ((), ()))
QSCALE = (D ** -0.5) * math.log2(math.e)


def _dft_mats():
    shp = (2, 128, 128)
    hf = lax.broadcasted_iota(jnp.int32, shp, 0)
    r = lax.broadcasted_iota(jnp.int32, shp, 1)
    j = lax.broadcasted_iota(jnp.int32, shp, 2)
    f = hf * 64 + (r & 63)
    k = ((2 * f + 1) * j + jnp.where(r >= 64, 128, 0)) & 511
    fm = jnp.cos(k.astype(F32) * (2 * math.pi / 512))
    ff = hf * 64 + (j & 63)
    k2 = ((2 * ff + 1) * (r + 128) + jnp.where(j >= 64, 128, 0)) & 511
    gm = jnp.cos(k2.astype(F32) * (2 * math.pi / 512)) * (1.0 / 128)
    return fm.astype(BF16), gm.astype(BF16)


U32 = jnp.uint32


def _pk(v):
    return pltpu.bitcast(v, U32)


def _up(v):
    return pltpu.bitcast(v, BF16)


def _own_block(trips, fn):
    def body(_, c):
        fn()
        return c
    lax.fori_loop(0, trips, body, 0)


def _spread(pieces, aux):
    n = len(pieces)
    done = 0
    for k, piece in enumerate(pieces):
        piece()
        tgt = (len(aux) * (k + 1)) // n
        while done < tgt:
            aux[done]()
            done += 1


def _kernel(x_h, c_h, wq_h, wuk_h, wuv_h, wo_h, bk_h, bv_h, sk_h, h_h, d_h, gw_h,
            o_h,
            x_v, c_v, wq_raw, wuk_raw, wuv_raw, wo_v, bk_s, bv_s, h_s,
            x_p, c_p, wq_s, wkv_s, q_s, k_s, v_s, ctx_s, kv_s, y_s, u_s, ht_s, f_s, g_s, o_s,
            sk_v, d_v, gw_v,
            sem_c, sem_x, sem_f, sem_g, sem_wo, sem_h, sem_small, sem_o):
    def cp_c(b):
        return pltpu.make_async_copy(c_h.at[pl.ds(b * RC, RC)], c_v.at[pl.ds(b * RC, RC)], sem_c.at[b])

    def cp_x(b):
        return pltpu.make_async_copy(x_h.at[pl.ds(b * RC, RC)], x_v.at[pl.ds(b * RC, RC)], sem_x.at[b])

    def cp_wq0(b):
        rows = pl.ds(b * 256, 256)
        return pltpu.make_async_copy(wq_h.at[rows, 0], wq_raw.at[0, rows], sem_f.at[b])

    def cp_wuk0(b):
        rows = pl.ds(b * 128, 128)
        return pltpu.make_async_copy(wuk_h.at[rows, 0], wuk_raw.at[0, rows], sem_f.at[4 + b])

    def cp_wuv0(b):
        rows = pl.ds(b * 128, 128)
        return pltpu.make_async_copy(wuv_h.at[rows, 0], wuv_raw.at[0, rows], sem_f.at[8 + b])

    def cp_b0(src, dst, pad, b, sem0):
        cg = b // 2
        r0 = (b % 2) * 1024
        return pltpu.make_async_copy(src.at[pl.ds(r0, 1024), pl.ds(cg * 128, 128)],
                                     dst.at[cg, pl.ds(pad + r0, 1024)], sem_f.at[sem0 + b])

    def cp_bk0(b):
        return cp_b0(bk_h, bk_s, PADK, b, 12)

    def cp_bv0(b):
        return cp_b0(bv_h, bv_s, 0, b, 16)

    def cp_h(g):
        return pltpu.make_async_copy(h_h.at[pl.ds(2 * g, 2)], h_s.at[pl.ds(2 * g, 2)], sem_h.at[g])

    def cp_wkv(g):
        return [pltpu.make_async_copy(wuk_h.at[:, g], wuk_raw.at[g], sem_g.at[g * 8]),
                pltpu.make_async_copy(wuv_h.at[:, g], wuv_raw.at[g], sem_g.at[g * 8 + 1])]

    def cp_kvaux(g):
        cps = [pltpu.make_async_copy(wq_h.at[:, g], wq_raw.at[g], sem_g.at[g * 8 + 2])]
        for u in range(2):
            cg = 2 * g + u
            cols = pl.ds(cg * 128, 128)
            cps.append(pltpu.make_async_copy(bk_h.at[:, cols], bk_s.at[cg, pl.ds(PADK, S)],
                                             sem_g.at[g * 8 + 3 + u]))
            cps.append(pltpu.make_async_copy(bv_h.at[:, cols], bv_s.at[cg], sem_g.at[g * 8 + 5 + u]))
        return cps

    cp_wo = pltpu.make_async_copy(wo_h, wo_v, sem_wo.at[0])
    cp_small = [pltpu.make_async_copy(sk_h, sk_v, sem_small.at[0]),
                pltpu.make_async_copy(d_h, d_v, sem_small.at[1]),
                pltpu.make_async_copy(gw_h, gw_v, sem_small.at[2])]

    def cp_o(r):
        rows = pl.ds(r * FO, FO)
        return pltpu.make_async_copy(o_s.at[rows], o_h.at[rows], sem_o.at[r])

    def start_kv0(b):
        cp_wq0(b).start()
        cp_bk0(b).start()
        cp_bv0(b).start()

    def relayout_wkv_step(g, b, s, which):
        m0 = pl.multiple_of(b * 128 + s * 32, 32)
        src = wuk_raw if which == 0 else wuv_raw
        t = jnp.swapaxes(src[g, pl.ds(m0, 32)], 0, 1)
        prow = pl.ds(pl.multiple_of(b * 64 + s * 16, 16), 16)
        for hh in range(HG):
            c0 = hh * 256 + which * 128
            wkv_s[prow, c0:c0 + 128] = _pk(t[hh])

    def stage_c(bn, rb):
        c_p[rb * 64:(rb + 1) * 64, :] = _pk(c_v[pl.ds(pl.multiple_of(bn * RC + rb * 128, 128), 128), :])

    def stage_x(bn, rb):
        x_p[rb * 64:(rb + 1) * 64, :] = _pk(x_v[pl.ds(pl.multiple_of(bn * RC + rb * 128, 128), 128), :])

    one = pl.semaphore_read(sem_o.at[0]) + 1
    for cp in cp_small:
        cp.start()
    for b in range(4):
        cp_wuk0(b).start()
        cp_wuv0(b).start()
    cp_c(0).start()

    fm, gm = _dft_mats()
    for hf in range(2):
        f_s[hf] = _pk(fm[hf])
        g_s[hf] = _pk(gm[hf])
    bk_s[:, 0:PADK, :] = jnp.zeros((NCG, PADK, 128), BF16)

    start_kv0(0)
    cp_c(1).start()

    for b in range(4):
        def wait_wkv0(b=b):
            cp_wuk0(b).wait()
            cp_wuv0(b).wait()
        _own_block(one, wait_wkv0)
        for s in range(4):
            relayout_wkv_step(0, b, s, 0)
            relayout_wkv_step(0, b, s, 1)

    def wait_rest():
        cp_small[0].wait()
        cp_c(0).wait()
    _own_block(one, wait_rest)
    for rb in range(RC // 128):
        stage_c(0, rb)

    def group_body(g, carry):
        @pl.when(g + 1 < NG)
        def _():
            for cp in cp_wkv(g + 1):
                cp.start()

        @pl.when(g == 1)
        def _():
            cp_wo.start()

        @pl.when(g > 0)
        def _():
            for cp in cp_kvaux(g):
                cp.wait()

        def kv_body(b, c2):
            p = g * 4 + b

            def dma_g0():
                @pl.when(b + 1 < NRC)
                def _():
                    cp_c(b + 1).wait()
                cp_wq0(b).wait()
                cp_bk0(b).wait()
                cp_bv0(b).wait()

                @pl.when(b + 1 < NRC)
                def _():
                    start_kv0(b + 1)

                @pl.when(b + 2 < NRC)
                def _():
                    cp_c(b + 2).start()

                @pl.when(b == 1)
                def _():
                    cp_x(0).start()
                    cp_x(1).start()
                    cp_h(0).start()

                @pl.when(b == 2)
                def _():
                    cp_x(2).start()
                    cp_x(3).start()
            _own_block((g == 0).astype(jnp.int32), dma_g0)
            bn = (b + 1) % NRC

            def mm_piece(rb, hh):
                def run():
                    prow = pl.ds(pl.multiple_of(b * (RC // 2) + rb * 64, 64), 64)
                    kk = jnp.dot(_up(c_p[rb * 64:(rb + 1) * 64, :]), _up(wkv_s[:, hh * 256:(hh + 1) * 256]),
                                 preferred_element_type=F32)
                    k_s[hh, prow, :] = _pk(kk[:, 0:128].astype(BF16))
                    v_s[hh, prow, :] = _pk(kk[:, 128:256].astype(BF16))
                return run

            def rq_step(s):
                def run():
                    m0 = pl.multiple_of(b * 256 + s * 32, 32)
                    t = jnp.swapaxes(wq_raw[g, pl.ds(m0, 32)], 0, 1)
                    prow = pl.ds(pl.multiple_of(b * 128 + s * 16, 16), 16)
                    for hh in range(HG):
                        wq_s[prow, hh * 128:(hh + 1) * 128] = _pk(t[hh])
                return run

            cg = p // 2
            rh = p % 2
            w = sk_v[:, pl.ds(pl.multiple_of(cg * 128, 128), 128)].astype(F32)

            def kvb_step(s):
                def run():
                    r0 = pl.multiple_of(rh * 1024 + s * 64, 64)
                    kw = bk_s[cg, pl.ds(r0, 64 + PADK), :].astype(F32)
                    acc = kw[PADK:] * w[0:1]
                    for j in range(1, 4):
                        acc = acc + kw[PADK - j:PADK - j + 64] * w[j:j + 1]
                    kvv = acc * bv_s[cg, pl.ds(r0, 64), :].astype(F32)
                    kv_s[cg, pl.ds(pl.multiple_of(rh * 512 + s * 32, 32), 32), :] = _pk(kvv.astype(BF16))
                return run

            aux = []
            for s in range(8):
                aux += [rq_step(s), kvb_step(2 * s), kvb_step(2 * s + 1)]
            k = 0
            done = 0
            for rb in range(RC // 128):
                for hh in range(HG):
                    mm_piece(rb, hh)()
                    k += 1
                    tgt = min(len(aux), (len(aux) * k) // 30)
                    while done < tgt:
                        aux[done]()
                        done += 1
                stage_c(bn, rb)
            return c2

        lax.fori_loop(0, NRC, kv_body, 0)

        def q_body(b, c2):
            bn = (b + 1) % NRC
            p = g * 4 + b
            cg = p // 2
            hf = p % 2

            def waits():
                @pl.when(jnp.logical_and(g == 0, b + 1 < NRC))
                def _():
                    cp_x(b + 1).wait()

                @pl.when(jnp.logical_and(g + 1 < NG, b == 0))
                def _():
                    for cp in cp_wkv(g + 1):
                        cp.wait()
            _own_block(jnp.logical_or(g == 0, b == 0).astype(jnp.int32), waits)

            gn = jnp.minimum(g + 1, NG - 1)
            fh = _up(f_s[hf])
            gh = _up(g_s[hf])
            st = {}

            def q_piece(rb, hh):
                def run():
                    prow = pl.ds(pl.multiple_of(b * (RC // 2) + rb * 64, 64), 64)
                    qq = jnp.dot(_up(x_p[rb * 64:(rb + 1) * 64, :]), _up(wq_s[:, hh * 128:(hh + 1) * 128]),
                                 preferred_element_type=F32) * QSCALE
                    q_s[hh, prow, :] = _pk(qq.astype(BF16))
                return run

            def u_piece(q):
                def run():
                    ucat = jnp.concatenate(
                        [_up(kv_s[cg, i * 64:(i + 1) * 64, :]) for i in range(4 * q, 4 * q + 4)], axis=1)
                    u_s[:, q * 512:(q + 1) * 512] = jnp.dot(fh, ucat, preferred_element_type=F32)
                return run

            def h_piece(q):
                def run():
                    hcat = jnp.concatenate(
                        [h_s[cg, :, m * CB:(m + 1) * CB] for m in range(4 * q, 4 * q + 4)], axis=0)
                    st["hh", q] = lax.dot_general(fh, hcat, NT, preferred_element_type=F32)
                return run

            sgn = jnp.where((lax.broadcasted_iota(jnp.int32, (64, 128), 0) & 1) == 0,
                            1.0, -1.0).astype(F32)

            def t_step(m):
                def run():
                    cur = st["hh", m // 4][:, (m % 4) * CB:(m % 4 + 1) * CB]
                    tr = sgn * cur[64:128]
                    ti = sgn * cur[0:64]
                    if m > 0:
                        prv = st["hh", (m - 1) // 4][:, ((m - 1) % 4) * CB:((m - 1) % 4 + 1) * CB]
                        tr = prv[0:64] + tr
                        ti = prv[64:128] - ti
                    else:
                        ti = -ti
                    ht_s[0:64, m * CB:(m + 1) * CB] = tr
                    ht_s[64:128, m * CB:(m + 1) * CB] = ti
                return run

            RB = 32

            def p_step(i, rb, m):
                def run():
                    a0 = (i - m) * CB
                    b0 = m * CB
                    ur = u_s[rb:rb + RB, a0:a0 + CB]
                    ui = u_s[64 + rb:64 + rb + RB, a0:a0 + CB]
                    hr = ht_s[rb:rb + RB, b0:b0 + CB]
                    hi = ht_s[64 + rb:64 + rb + RB, b0:b0 + CB]
                    pr = ur * hr - ui * hi
                    pi = ur * hi + ui * hr
                    if m > 0:
                        pr = st["yr"] + pr
                        pi = st["yi"] + pi
                    st["yr"], st["yi"] = pr, pi
                    if m == i:
                        st["Y", i, rb] = (pr.astype(BF16), pi.astype(BF16))
                return run

            def i_piece(q):
                def run():
                    blocks = []
                    for i in range(4 * q, 4 * q + 4):
                        parts = [st.pop(("Y", i, rb)) for rb in range(0, 64, RB)]
                        blocks.append(jnp.concatenate([t[0] for t in parts] + [t[1] for t in parts], axis=0))
                    st["yo", q] = jnp.dot(gh, jnp.concatenate(blocks, axis=1), preferred_element_type=F32)
                return run

            def y_step(i):
                def run():
                    yo = st["yo", i // 4][:, (i % 4) * CB:(i % 4 + 1) * CB]
                    old = jnp.where(hf == 0, 0.0, y_s[cg, i * CB:(i + 1) * CB, :])
                    y_s[cg, i * CB:(i + 1) * CB, :] = old + yo
                return run

            rsteps = [(lambda s=s, wh=wh: relayout_wkv_step(gn, b, s, wh)) for s in range(4) for wh in range(2)]
            for q in range(4):
                u_piece(q)()
            for q in range(4):
                h_piece(q)()
            qp = [q_piece(rb, hh) for rb in range(RC // 128) for hh in range(HG)]
            aux = [t_step(m) for m in range(NCB)]
            psteps = [(i, rb, m) for i in range(NCB) for rb in range(0, 64, RB) for m in range(i + 1)]
            NQ1 = 28
            per = len(psteps) / float(NQ1 - 1)
            done = 0
            pend_i = [0, 1, 2, 3]
            pend_y = []
            for k in range(len(qp)):
                qp[k]()
                if k % HG == HG - 1:
                    stage_x(bn, k // HG)
                if k == 0:
                    for a in aux:
                        a()
                    continue
                while pend_i and done >= 2 * sum(range(1, 4 * pend_i[0] + 5)):
                    q = pend_i.pop(0)
                    i_piece(q)()
                    pend_y += list(range(4 * q, 4 * q + 4))
                    break
                tgt = min(len(psteps), int(round(per * k)))
                while done < tgt:
                    p_step(*psteps[done])()
                    done += 1
                if k % 3 == 2 and rsteps:
                    rsteps.pop(0)()
                ny = 1 if pend_i else 2
                for _ in range(ny):
                    if pend_y:
                        y_step(pend_y.pop(0))()
            assert not pend_i and not rsteps
            while pend_y:
                y_step(pend_y.pop(0))()
            return c2

        @pl.when(g + 1 < NG)
        def _():
            for cp in cp_kvaux(g + 1):
                cp.start()
            cp_h(g + 1).start()

        cp_h(g).wait()

        @pl.when(g == 0)
        def _():
            cp_x(0).wait()
            for rb in range(RC // 128):
                stage_x(0, rb)

        lax.fori_loop(0, NRC, q_body, 0)

        mask = (lax.broadcasted_iota(jnp.int32, (BQ, BQ), 1)
                <= lax.broadcasted_iota(jnp.int32, (BQ, BQ), 0))
        HB = BQ // 2

        def attn_body(t, c2):
            def qk(hh, i, z):
                q = q_s[hh, i * HB:(i + 1) * HB, :]
                if z is not None:
                    q = jnp.concatenate([q[0:8] + z, q[8:]], axis=0)
                return lax.dot_general(_up(q), _up(k_s[hh, 0:(i + 1) * HB, :]), NT,
                                       preferred_element_type=F32)

            def sm(i, s):
                L = (i + 1) * BQ
                sd = jnp.where(mask, s[:, L - BQ:], NEG)
                s = jnp.concatenate([s[:, :L - BQ], sd], axis=1) if i > 0 else sd
                m = jnp.max(s, axis=1, keepdims=True)
                p = jnp.exp2(s - m)
                l = jnp.sum(p, axis=1, keepdims=True)
                return p.astype(BF16), l

            def pv(hh, i, p):
                return jnp.dot(p, _up(v_s[hh, 0:(i + 1) * HB, :]), preferred_element_type=F32)

            def fin(hh, i, ctx, l):
                r = pl.reciprocal(l, approx=True)
                r = r * (2.0 - l * r)
                o = _pk((ctx * r).astype(BF16))
                ctx_s[g * HG + hh, i * HB:(i + 1) * HB, :] = o
                a = o[0:8]
                for kk in range(1, 8):
                    a = a | o[8 * kk:8 * kk + 8]
                return (a & 1) >> 1

            order = []
            for i in range(NBQ // 2):
                for u in range(0, AH, 2):
                    ha, hb = AH * t + u, AH * t + u + 1
                    order += [(ha, NBQ - 1 - i), (hb, NBQ - 1 - i), (hb, i), (ha, i)]
            n = len(order)
            lag = 3
            ss, cs, zs = {}, {}, {}
            ss[0] = qk(*order[0], None)
            for j in range(n + lag):
                if j + 1 < n:
                    ss[j + 1] = qk(*order[j + 1], zs.pop(j + 1, None))
                if j < n:
                    p, l = sm(order[j][1], ss.pop(j))
                    cs[j] = (pv(*order[j], p), l)
                if 0 <= j - lag < n:
                    zs[j + 2] = fin(*order[j - lag], *cs.pop(j - lag))
            return c2

        lax.fori_loop(0, HG // AH, attn_body, 0)
        return carry

    lax.fori_loop(0, NG, group_body, 0)

    cp_wo.wait()
    cp_small[1].wait()
    cp_small[2].wait()

    def out_body(r, carry):
        rows = pl.ds(pl.multiple_of(r * FO, FO), FO)
        prow = pl.ds(pl.multiple_of(r * (FO // 2), FO // 2), FO // 2)
        ctx = jnp.concatenate([_up(ctx_s[hh, prow, :]) for hh in range(H)], axis=1)
        a = jnp.dot(ctx, wo_v[...], preferred_element_type=F32)
        xf = x_v[rows, :].astype(F32)
        gw = gw_v[...].astype(F32)[None, :]
        gate = jax.nn.sigmoid(jnp.sum(xf * gw, axis=1, keepdims=True))
        dd = d_v[...].astype(F32)[None, :]
        for cg in range(NCG):
            cols = slice(cg * 128, (cg + 1) * 128)
            yb = y_s[cg, rows, :] + _up(kv_s[cg, prow, :]).astype(F32) * dd[:, cols]
            o_s[rows, cols] = (gate * a[:, cols] + (1.0 - gate) * (xf[:, cols] * yb)).astype(BF16)
        cp_o(r).start()
        return carry

    lax.fori_loop(0, S // FO, out_body, 0)
    for r in range(S // FO):
        cp_o(r).wait()


@jax.jit
def pallas_gated_mix__compressed_kv_cla__ssm_conv_h3__prompt_kernel(
    A_x: jax.Array,
    A_c_kv: jax.Array,
    A_w_q: jax.Array,
    A_w_uk: jax.Array,
    A_w_uv: jax.Array,
    A_w_o: jax.Array,
    B_q: jax.Array,
    B_k: jax.Array,
    B_v: jax.Array,
    B_shift_k: jax.Array,
    B_ssm_k: jax.Array,
    B_ssm_D: jax.Array,
    gate_w: jax.Array,
):
    del B_q
    x = A_x.reshape(S, M)
    c = A_c_kv.reshape(S, DC)
    wq = A_w_q.reshape(M, NG, HG, D)
    wuk = A_w_uk.reshape(DC, NG, HG, D)
    wuv = A_w_uv.reshape(DC, NG, HG, D)
    wo = A_w_o.reshape(H * D, M)
    bk = B_k.reshape(S, M)
    bv = B_v.reshape(S, M)
    skt = B_shift_k.T
    hk = B_ssm_k.reshape(NCG, 128, S)

    dma = pltpu.SemaphoreType.DMA
    scratch = [
        pltpu.VMEM((S, M), BF16),
        pltpu.VMEM((S, DC), BF16),
        pltpu.VMEM((NG, M, HG, D), BF16),
        pltpu.VMEM((NG, DC, HG, D), BF16),
        pltpu.VMEM((NG, DC, HG, D), BF16),
        pltpu.VMEM((H * D, M), BF16),
        pltpu.VMEM((NCG, PADK + S, 128), BF16),
        pltpu.VMEM((NCG, S, 128), BF16),
        pltpu.VMEM((NCG, 128, S), BF16),
        pltpu.VMEM((RC // 2, M), U32),
        pltpu.VMEM((RC // 2, DC), U32),
        pltpu.VMEM((M // 2, HG * D), U32),
        pltpu.VMEM((DC // 2, 2 * HG * D), U32),
        pltpu.VMEM((HG, S // 2, D), U32),
        pltpu.VMEM((HG, S // 2, D), U32),
        pltpu.VMEM((HG, S // 2, D), U32),
        pltpu.VMEM((H, S // 2, D), U32),
        pltpu.VMEM((NCG, S // 2, 128), U32),
        pltpu.VMEM((NCG, S, 128), F32),
        pltpu.VMEM((128, S), F32),
        pltpu.VMEM((128, S), F32),
        pltpu.VMEM((2, 64, 128), U32),
        pltpu.VMEM((2, 64, 128), U32),
        pltpu.VMEM((S, M), BF16),
        pltpu.VMEM((4, M), BF16),
        pltpu.VMEM((M,), BF16),
        pltpu.VMEM((M,), BF16),
        dma((4,)), dma((4,)), dma((20,)), dma((NG * 8,)), dma((1,)), dma((NG,)), dma((3,)),
        dma((S // FO,)),
    ]
    out = pl.pallas_call(
        _kernel,
        out_shape=jax.ShapeDtypeStruct((S, M), BF16),
        in_specs=[pl.BlockSpec(memory_space=pl.ANY)] * 12,
        out_specs=pl.BlockSpec(memory_space=pl.ANY),
        scratch_shapes=scratch,
        compiler_params=pltpu.CompilerParams(vmem_limit_bytes=120 * 1024 * 1024),
    )(x, c, wq, wuk, wuv, wo, bk, bv, skt, hk, B_ssm_D, gate_w)
    return out.reshape(1, S, M)
```

```python
import math

import jax
import jax.numpy as jnp
from jax import lax
import jax.experimental.pallas as pl
import jax.experimental.pallas.tpu as pltpu

F32 = jnp.float32
BF16 = jnp.bfloat16

S = 2048
M = 1024
H = 32
D = 128
DC = 512
HG = 8
NG = H // HG
RC = 512
NRC = S // RC
BQ = 128
NBQ = S // BQ
AH = 2
CB = 128
NCB = S // CB
NCG = M // 128
FO = 256
PADK = 16
NEG = -1e9
NT = (((1,), (1,)), ((), ()))
QSCALE = (D ** -0.5) * math.log2(math.e)


def _dft_mats():
    shp = (2, 128, 128)
    hf = lax.broadcasted_iota(jnp.int32, shp, 0)
    r = lax.broadcasted_iota(jnp.int32, shp, 1)
    j = lax.broadcasted_iota(jnp.int32, shp, 2)
    f = hf * 64 + (r & 63)
    k = ((2 * f + 1) * j + jnp.where(r >= 64, 128, 0)) & 511
    fm = jnp.cos(k.astype(F32) * (2 * math.pi / 512))
    ff = hf * 64 + (j & 63)
    k2 = ((2 * ff + 1) * (r + 128) + jnp.where(j >= 64, 128, 0)) & 511
    gm = jnp.cos(k2.astype(F32) * (2 * math.pi / 512)) * (1.0 / 128)
    return fm.astype(BF16), gm.astype(BF16)


U32 = jnp.uint32


def _pk(v):
    return pltpu.bitcast(v, U32)


def _up(v):
    return pltpu.bitcast(v, BF16)


def _own_block(trips, fn):
    def body(_, c):
        fn()
        return c
    lax.fori_loop(0, trips, body, 0)


def _spread(pieces, aux):
    n = len(pieces)
    done = 0
    for k, piece in enumerate(pieces):
        piece()
        tgt = (len(aux) * (k + 1)) // n
        while done < tgt:
            aux[done]()
            done += 1


def _kernel(x_h, c_h, wq_h, wuk_h, wuv_h, wo_h, bk_h, bv_h, sk_h, h_h, d_h, gw_h,
            o_h,
            x_v, c_v, wq_raw, wuk_raw, wuv_raw, wo_v, bk_s, bv_s, h_s,
            x_p, c_p, wq_s, wkv_s, q_s, k_s, v_s, ctx_s, kv_s, y_s, u_s, ht_s, f_s, g_s, o_s,
            sk_v, d_v, gw_v,
            sem_c, sem_x, sem_f, sem_g, sem_wo, sem_h, sem_small, sem_o):
    def cp_c(b):
        return pltpu.make_async_copy(c_h.at[pl.ds(b * RC, RC)], c_v.at[pl.ds(b * RC, RC)], sem_c.at[b])

    def cp_x(b):
        return pltpu.make_async_copy(x_h.at[pl.ds(b * RC, RC)], x_v.at[pl.ds(b * RC, RC)], sem_x.at[b])

    def cp_wq0(b):
        rows = pl.ds(b * 256, 256)
        return pltpu.make_async_copy(wq_h.at[rows, 0], wq_raw.at[0, rows], sem_f.at[b])

    def cp_wuk0(b):
        rows = pl.ds(b * 128, 128)
        return pltpu.make_async_copy(wuk_h.at[rows, 0], wuk_raw.at[0, rows], sem_f.at[4 + b])

    def cp_wuv0(b):
        rows = pl.ds(b * 128, 128)
        return pltpu.make_async_copy(wuv_h.at[rows, 0], wuv_raw.at[0, rows], sem_f.at[8 + b])

    def cp_b0(src, dst, pad, b, sem0):
        cg = b // 2
        r0 = (b % 2) * 1024
        return pltpu.make_async_copy(src.at[pl.ds(r0, 1024), pl.ds(cg * 128, 128)],
                                     dst.at[cg, pl.ds(pad + r0, 1024)], sem_f.at[sem0 + b])

    def cp_bk0(b):
        return cp_b0(bk_h, bk_s, PADK, b, 12)

    def cp_bv0(b):
        return cp_b0(bv_h, bv_s, 0, b, 16)

    def cp_h(g):
        return pltpu.make_async_copy(h_h.at[pl.ds(2 * g, 2)], h_s.at[pl.ds(2 * g, 2)], sem_h.at[g])

    def cp_wkv(g):
        return [pltpu.make_async_copy(wuk_h.at[:, g], wuk_raw.at[g], sem_g.at[g * 8]),
                pltpu.make_async_copy(wuv_h.at[:, g], wuv_raw.at[g], sem_g.at[g * 8 + 1])]

    def cp_kvaux(g):
        cps = [pltpu.make_async_copy(wq_h.at[:, g], wq_raw.at[g], sem_g.at[g * 8 + 2])]
        for u in range(2):
            cg = 2 * g + u
            cols = pl.ds(cg * 128, 128)
            cps.append(pltpu.make_async_copy(bk_h.at[:, cols], bk_s.at[cg, pl.ds(PADK, S)],
                                             sem_g.at[g * 8 + 3 + u]))
            cps.append(pltpu.make_async_copy(bv_h.at[:, cols], bv_s.at[cg], sem_g.at[g * 8 + 5 + u]))
        return cps

    cp_wo = pltpu.make_async_copy(wo_h, wo_v, sem_wo.at[0])
    cp_small = [pltpu.make_async_copy(sk_h, sk_v, sem_small.at[0]),
                pltpu.make_async_copy(d_h, d_v, sem_small.at[1]),
                pltpu.make_async_copy(gw_h, gw_v, sem_small.at[2])]

    def cp_o(r):
        rows = pl.ds(r * FO, FO)
        return pltpu.make_async_copy(o_s.at[rows], o_h.at[rows], sem_o.at[r])

    def start_kv0(b):
        cp_wq0(b).start()
        cp_bk0(b).start()
        cp_bv0(b).start()

    def relayout_wkv_step(g, b, s, which):
        m0 = pl.multiple_of(b * 128 + s * 32, 32)
        src = wuk_raw if which == 0 else wuv_raw
        t = jnp.swapaxes(src[g, pl.ds(m0, 32)], 0, 1)
        prow = pl.ds(pl.multiple_of(b * 64 + s * 16, 16), 16)
        for hh in range(HG):
            c0 = hh * 256 + which * 128
            wkv_s[prow, c0:c0 + 128] = _pk(t[hh])

    def stage_c(bn, rb):
        c_p[rb * 64:(rb + 1) * 64, :] = _pk(c_v[pl.ds(pl.multiple_of(bn * RC + rb * 128, 128), 128), :])

    def stage_x(bn, rb):
        x_p[rb * 64:(rb + 1) * 64, :] = _pk(x_v[pl.ds(pl.multiple_of(bn * RC + rb * 128, 128), 128), :])

    for cp in cp_small:
        cp.start()
    for b in range(4):
        cp_wuk0(b).start()
        cp_wuv0(b).start()
    cp_c(0).start()

    fm, gm = _dft_mats()
    for hf in range(2):
        f_s[hf] = _pk(fm[hf])
        g_s[hf] = _pk(gm[hf])
    bk_s[:, 0:PADK, :] = jnp.zeros((NCG, PADK, 128), BF16)

    start_kv0(0)
    cp_c(1).start()

    for b in range(4):
        cp_wuk0(b).wait()
        cp_wuv0(b).wait()
        for s in range(4):
            relayout_wkv_step(0, b, s, 0)
            relayout_wkv_step(0, b, s, 1)

    cp_small[0].wait()
    cp_c(0).wait()
    for rb in range(RC // 128):
        stage_c(0, rb)

    def group_body(g, carry):
        @pl.when(g + 1 < NG)
        def _():
            for cp in cp_wkv(g + 1):
                cp.start()

        @pl.when(g == 1)
        def _():
            cp_wo.start()

        @pl.when(g > 0)
        def _():
            for cp in cp_kvaux(g):
                cp.wait()

        def kv_body(b, c2):
            p = g * 4 + b

            def dma_g0():
                @pl.when(b + 1 < NRC)
                def _():
                    cp_c(b + 1).wait()
                cp_wq0(b).wait()
                cp_bk0(b).wait()
                cp_bv0(b).wait()

                @pl.when(b + 1 < NRC)
                def _():
                    start_kv0(b + 1)

                @pl.when(b + 2 < NRC)
                def _():
                    cp_c(b + 2).start()

                @pl.when(b == 1)
                def _():
                    cp_x(0).start()
                    cp_x(1).start()
                    cp_h(0).start()

                @pl.when(b == 2)
                def _():
                    cp_x(2).start()
                    cp_x(3).start()
            _own_block((g == 0).astype(jnp.int32), dma_g0)
            bn = (b + 1) % NRC

            def mm_piece(rb, hh):
                def run():
                    prow = pl.ds(pl.multiple_of(b * (RC // 2) + rb * 64, 64), 64)
                    kk = jnp.dot(_up(c_p[rb * 64:(rb + 1) * 64, :]), _up(wkv_s[:, hh * 256:(hh + 1) * 256]),
                                 preferred_element_type=F32)
                    k_s[hh, prow, :] = _pk(kk[:, 0:128].astype(BF16))
                    v_s[hh, prow, :] = _pk(kk[:, 128:256].astype(BF16))
                return run

            def rq_step(s):
                def run():
                    m0 = pl.multiple_of(b * 256 + s * 32, 32)
                    t = jnp.swapaxes(wq_raw[g, pl.ds(m0, 32)], 0, 1)
                    prow = pl.ds(pl.multiple_of(b * 128 + s * 16, 16), 16)
                    for hh in range(HG):
                        wq_s[prow, hh * 128:(hh + 1) * 128] = _pk(t[hh])
                return run

            cg = p // 2
            rh = p % 2
            w = sk_v[:, pl.ds(pl.multiple_of(cg * 128, 128), 128)].astype(F32)

            def kvb_step(s):
                def run():
                    r0 = pl.multiple_of(rh * 1024 + s * 64, 64)
                    kw = bk_s[cg, pl.ds(r0, 64 + PADK), :].astype(F32)
                    acc = kw[PADK:] * w[0:1]
                    for j in range(1, 4):
                        acc = acc + kw[PADK - j:PADK - j + 64] * w[j:j + 1]
                    kvv = acc * bv_s[cg, pl.ds(r0, 64), :].astype(F32)
                    kv_s[cg, pl.ds(pl.multiple_of(rh * 512 + s * 32, 32), 32), :] = _pk(kvv.astype(BF16))
                return run

            aux = []
            for s in range(8):
                aux += [rq_step(s), kvb_step(2 * s), kvb_step(2 * s + 1)]
            k = 0
            done = 0
            for rb in range(RC // 128):
                for hh in range(HG):
                    mm_piece(rb, hh)()
                    k += 1
                    tgt = min(len(aux), (len(aux) * k) // 30)
                    while done < tgt:
                        aux[done]()
                        done += 1
                stage_c(bn, rb)
            return c2

        lax.fori_loop(0, NRC, kv_body, 0)

        def q_body(b, c2):
            bn = (b + 1) % NRC
            p = g * 4 + b
            cg = p // 2
            hf = p % 2

            def waits():
                @pl.when(jnp.logical_and(g == 0, b + 1 < NRC))
                def _():
                    cp_x(b + 1).wait()

                @pl.when(jnp.logical_and(g + 1 < NG, b == 0))
                def _():
                    for cp in cp_wkv(g + 1):
                        cp.wait()
            _own_block(jnp.logical_or(g == 0, b == 0).astype(jnp.int32), waits)

            gn = jnp.minimum(g + 1, NG - 1)
            fh = _up(f_s[hf])
            gh = _up(g_s[hf])
            st = {}

            def q_piece(rb, hh):
                def run():
                    prow = pl.ds(pl.multiple_of(b * (RC // 2) + rb * 64, 64), 64)
                    qq = jnp.dot(_up(x_p[rb * 64:(rb + 1) * 64, :]), _up(wq_s[:, hh * 128:(hh + 1) * 128]),
                                 preferred_element_type=F32) * QSCALE
                    q_s[hh, prow, :] = _pk(qq.astype(BF16))
                return run

            def u_piece(q):
                def run():
                    ucat = jnp.concatenate(
                        [_up(kv_s[cg, i * 64:(i + 1) * 64, :]) for i in range(4 * q, 4 * q + 4)], axis=1)
                    u_s[:, q * 512:(q + 1) * 512] = jnp.dot(fh, ucat, preferred_element_type=F32)
                return run

            def h_piece(q):
                def run():
                    hcat = jnp.concatenate(
                        [h_s[cg, :, m * CB:(m + 1) * CB] for m in range(4 * q, 4 * q + 4)], axis=0)
                    st["hh", q] = lax.dot_general(fh, hcat, NT, preferred_element_type=F32)
                return run

            sgn = jnp.where((lax.broadcasted_iota(jnp.int32, (64, 128), 0) & 1) == 0,
                            1.0, -1.0).astype(F32)

            def t_step(m):
                def run():
                    cur = st["hh", m // 4][:, (m % 4) * CB:(m % 4 + 1) * CB]
                    tr = sgn * cur[64:128]
                    ti = sgn * cur[0:64]
                    if m > 0:
                        prv = st["hh", (m - 1) // 4][:, ((m - 1) % 4) * CB:((m - 1) % 4 + 1) * CB]
                        tr = prv[0:64] + tr
                        ti = prv[64:128] - ti
                    else:
                        ti = -ti
                    ht_s[0:64, m * CB:(m + 1) * CB] = tr
                    ht_s[64:128, m * CB:(m + 1) * CB] = ti
                return run

            RB = 32

            def p_step(i, rb, m):
                def run():
                    a0 = (i - m) * CB
                    b0 = m * CB
                    ur = u_s[rb:rb + RB, a0:a0 + CB]
                    ui = u_s[64 + rb:64 + rb + RB, a0:a0 + CB]
                    hr = ht_s[rb:rb + RB, b0:b0 + CB]
                    hi = ht_s[64 + rb:64 + rb + RB, b0:b0 + CB]
                    pr = ur * hr - ui * hi
                    pi = ur * hi + ui * hr
                    if m > 0:
                        pr = st["yr"] + pr
                        pi = st["yi"] + pi
                    st["yr"], st["yi"] = pr, pi
                    if m == i:
                        st["Y", i, rb] = (pr.astype(BF16), pi.astype(BF16))
                return run

            def i_piece(q):
                def run():
                    blocks = []
                    for i in range(4 * q, 4 * q + 4):
                        parts = [st.pop(("Y", i, rb)) for rb in range(0, 64, RB)]
                        blocks.append(jnp.concatenate([t[0] for t in parts] + [t[1] for t in parts], axis=0))
                    st["yo", q] = jnp.dot(gh, jnp.concatenate(blocks, axis=1), preferred_element_type=F32)
                return run

            def y_step(i):
                def run():
                    yo = st["yo", i // 4][:, (i % 4) * CB:(i % 4 + 1) * CB]
                    old = jnp.where(hf == 0, 0.0, y_s[cg, i * CB:(i + 1) * CB, :])
                    y_s[cg, i * CB:(i + 1) * CB, :] = old + yo
                return run

            rsteps = [(lambda s=s, wh=wh: relayout_wkv_step(gn, b, s, wh)) for s in range(4) for wh in range(2)]
            for q in range(4):
                u_piece(q)()
            for q in range(4):
                h_piece(q)()
            qp = [q_piece(rb, hh) for rb in range(RC // 128) for hh in range(HG)]
            aux = [t_step(m) for m in range(NCB)]
            psteps = [(i, rb, m) for i in range(NCB) for rb in range(0, 64, RB) for m in range(i + 1)]
            NQ1 = 31
            per = len(psteps) / float(NQ1 - 1)
            done = 0
            pend_i = [0, 1, 2, 3]
            pend_y = []
            for k in range(len(qp)):
                qp[k]()
                if k % HG == HG - 1:
                    stage_x(bn, k // HG)
                if k == 0:
                    for a in aux:
                        a()
                    continue
                while pend_i and done >= 2 * sum(range(1, 4 * pend_i[0] + 5)):
                    q = pend_i.pop(0)
                    i_piece(q)()
                    pend_y += list(range(4 * q, 4 * q + 4))
                    break
                tgt = min(len(psteps), int(round(per * k)))
                while done < tgt:
                    p_step(*psteps[done])()
                    done += 1
                if k >= 22 and rsteps:
                    rsteps.pop(0)()
                ny = 1 if pend_i else 2
                for _ in range(ny):
                    if pend_y:
                        y_step(pend_y.pop(0))()
            assert not pend_i and not rsteps
            while pend_y:
                y_step(pend_y.pop(0))()
            return c2

        @pl.when(g + 1 < NG)
        def _():
            for cp in cp_kvaux(g + 1):
                cp.start()
            cp_h(g + 1).start()

        cp_h(g).wait()

        @pl.when(g == 0)
        def _():
            cp_x(0).wait()
            for rb in range(RC // 128):
                stage_x(0, rb)

        lax.fori_loop(0, NRC, q_body, 0)

        mask = (lax.broadcasted_iota(jnp.int32, (BQ, BQ), 1)
                <= lax.broadcasted_iota(jnp.int32, (BQ, BQ), 0))
        HB = BQ // 2

        def attn_body(t, c2):
            def qk(hh, i, z):
                q = q_s[hh, i * HB:(i + 1) * HB, :]
                if z is not None:
                    q = jnp.concatenate([q[0:8] + z, q[8:]], axis=0)
                return lax.dot_general(_up(q), _up(k_s[hh, 0:(i + 1) * HB, :]), NT,
                                       preferred_element_type=F32)

            def sm(i, s):
                L = (i + 1) * BQ
                sd = jnp.where(mask, s[:, L - BQ:], NEG)
                s = jnp.concatenate([s[:, :L - BQ], sd], axis=1) if i > 0 else sd
                m = jnp.max(s, axis=1, keepdims=True)
                p = jnp.exp2(s - m)
                l = jnp.sum(p, axis=1, keepdims=True)
                return p.astype(BF16), l

            def pv(hh, i, p):
                return jnp.dot(p, _up(v_s[hh, 0:(i + 1) * HB, :]), preferred_element_type=F32)

            def fin(hh, i, ctx, l):
                r = pl.reciprocal(l, approx=True)
                r = r * (2.0 - l * r)
                o = _pk((ctx * r).astype(BF16))
                ctx_s[g * HG + hh, i * HB:(i + 1) * HB, :] = o
                a = o[0:8]
                for kk in range(1, 8):
                    a = a | o[8 * kk:8 * kk + 8]
                return (a & 1) >> 1

            order = []
            for i in range(NBQ // 2):
                big, small = NBQ // 2 + i, (i + NBQ // 4) % (NBQ // 2)
                for u in range(0, AH, 2):
                    ha, hb = AH * t + u, AH * t + u + 1
                    order += [(ha, big), (hb, big), (hb, small), (ha, small)]
            n = len(order)
            lag = 3
            ss, cs, zs = {}, {}, {}
            ss[0] = qk(*order[0], None)
            for j in range(n + lag):
                if j + 1 < n:
                    ss[j + 1] = qk(*order[j + 1], zs.pop(j + 1, None))
                if j < n:
                    p, l = sm(order[j][1], ss.pop(j))
                    cs[j] = (pv(*order[j], p), l)
                if 0 <= j - lag < n:
                    zs[j + 2] = fin(*order[j - lag], *cs.pop(j - lag))
            return c2

        lax.fori_loop(0, HG // AH, attn_body, 0)
        return carry

    lax.fori_loop(0, NG, group_body, 0)

    cp_wo.wait()
    cp_small[1].wait()
    cp_small[2].wait()

    def out_body(r, carry):
        rows = pl.ds(pl.multiple_of(r * FO, FO), FO)
        prow = pl.ds(pl.multiple_of(r * (FO // 2), FO // 2), FO // 2)
        ctx = jnp.concatenate([_up(ctx_s[hh, prow, :]) for hh in range(H)], axis=1)
        a = jnp.dot(ctx, wo_v[...], preferred_element_type=F32)
        xf = x_v[rows, :].astype(F32)
        gw = gw_v[...].astype(F32)[None, :]
        gate = jax.nn.sigmoid(jnp.sum(xf * gw, axis=1, keepdims=True))
        dd = d_v[...].astype(F32)[None, :]
        for cg in range(NCG):
            cols = slice(cg * 128, (cg + 1) * 128)
            yb = y_s[cg, rows, :] + _up(kv_s[cg, prow, :]).astype(F32) * dd[:, cols]
            o_s[rows, cols] = (gate * a[:, cols] + (1.0 - gate) * (xf[:, cols] * yb)).astype(BF16)
        cp_o(r).start()
        return carry

    lax.fori_loop(0, S // FO, out_body, 0)
    for r in range(S // FO):
        cp_o(r).wait()


@jax.jit
def pallas_gated_mix__compressed_kv_cla__ssm_conv_h3__prompt_kernel(
    A_x: jax.Array,
    A_c_kv: jax.Array,
    A_w_q: jax.Array,
    A_w_uk: jax.Array,
    A_w_uv: jax.Array,
    A_w_o: jax.Array,
    B_q: jax.Array,
    B_k: jax.Array,
    B_v: jax.Array,
    B_shift_k: jax.Array,
    B_ssm_k: jax.Array,
    B_ssm_D: jax.Array,
    gate_w: jax.Array,
):
    del B_q
    x = A_x.reshape(S, M)
    c = A_c_kv.reshape(S, DC)
    wq = A_w_q.reshape(M, NG, HG, D)
    wuk = A_w_uk.reshape(DC, NG, HG, D)
    wuv = A_w_uv.reshape(DC, NG, HG, D)
    wo = A_w_o.reshape(H * D, M)
    bk = B_k.reshape(S, M)
    bv = B_v.reshape(S, M)
    skt = B_shift_k.T
    hk = B_ssm_k.reshape(NCG, 128, S)

    dma = pltpu.SemaphoreType.DMA
    scratch = [
        pltpu.VMEM((S, M), BF16),
        pltpu.VMEM((S, DC), BF16),
        pltpu.VMEM((NG, M, HG, D), BF16),
        pltpu.VMEM((NG, DC, HG, D), BF16),
        pltpu.VMEM((NG, DC, HG, D), BF16),
        pltpu.VMEM((H * D, M), BF16),
        pltpu.VMEM((NCG, PADK + S, 128), BF16),
        pltpu.VMEM((NCG, S, 128), BF16),
        pltpu.VMEM((NCG, 128, S), BF16),
        pltpu.VMEM((RC // 2, M), U32),
        pltpu.VMEM((RC // 2, DC), U32),
        pltpu.VMEM((M // 2, HG * D), U32),
        pltpu.VMEM((DC // 2, 2 * HG * D), U32),
        pltpu.VMEM((HG, S // 2, D), U32),
        pltpu.VMEM((HG, S // 2, D), U32),
        pltpu.VMEM((HG, S // 2, D), U32),
        pltpu.VMEM((H, S // 2, D), U32),
        pltpu.VMEM((NCG, S // 2, 128), U32),
        pltpu.VMEM((NCG, S, 128), F32),
        pltpu.VMEM((128, S), F32),
        pltpu.VMEM((128, S), F32),
        pltpu.VMEM((2, 64, 128), U32),
        pltpu.VMEM((2, 64, 128), U32),
        pltpu.VMEM((S, M), BF16),
        pltpu.VMEM((4, M), BF16),
        pltpu.VMEM((M,), BF16),
        pltpu.VMEM((M,), BF16),
        dma((4,)), dma((4,)), dma((20,)), dma((NG * 8,)), dma((1,)), dma((NG,)), dma((3,)),
        dma((S // FO,)),
    ]
    out = pl.pallas_call(
        _kernel,
        out_shape=jax.ShapeDtypeStruct((S, M), BF16),
        in_specs=[pl.BlockSpec(memory_space=pl.ANY)] * 12,
        out_specs=pl.BlockSpec(memory_space=pl.ANY),
        scratch_shapes=scratch,
        compiler_params=pltpu.CompilerParams(vmem_limit_bytes=120 * 1024 * 1024),
    )(x, c, wq, wuk, wuv, wo, bk, bv, skt, hk, B_ssm_D, gate_w)
    return out.reshape(1, S, M)
```

```python
import math

import jax
import jax.numpy as jnp
from jax import lax
import jax.experimental.pallas as pl
import jax.experimental.pallas.tpu as pltpu

F32 = jnp.float32
BF16 = jnp.bfloat16

S = 2048
M = 1024
H = 32
D = 128
DC = 512
HG = 8
NG = H // HG
RC = 512
NRC = S // RC
BQ = 128
NBQ = S // BQ
AH = 2
CB = 128
NCB = S // CB
NCG = M // 128
FO = 256
PADK = 16
NEG = -1e9
NT = (((1,), (1,)), ((), ()))
QSCALE = (D ** -0.5) * math.log2(math.e)


def _dft_mats():
    shp = (2, 128, 128)
    hf = lax.broadcasted_iota(jnp.int32, shp, 0)
    r = lax.broadcasted_iota(jnp.int32, shp, 1)
    j = lax.broadcasted_iota(jnp.int32, shp, 2)
    f = hf * 64 + (r & 63)
    k = ((2 * f + 1) * j + jnp.where(r >= 64, 128, 0)) & 511
    fm = jnp.cos(k.astype(F32) * (2 * math.pi / 512))
    ff = hf * 64 + (j & 63)
    k2 = ((2 * ff + 1) * (r + 128) + jnp.where(j >= 64, 128, 0)) & 511
    gm = jnp.cos(k2.astype(F32) * (2 * math.pi / 512)) * (1.0 / 128)
    return fm.astype(BF16), gm.astype(BF16)


U32 = jnp.uint32


def _pk(v):
    return pltpu.bitcast(v, U32)


def _up(v):
    return pltpu.bitcast(v, BF16)


def _own_block(trips, fn):
    def body(_, c):
        fn()
        return c
    lax.fori_loop(0, trips, body, 0)


def _spread(pieces, aux):
    n = len(pieces)
    done = 0
    for k, piece in enumerate(pieces):
        piece()
        tgt = (len(aux) * (k + 1)) // n
        while done < tgt:
            aux[done]()
            done += 1


def _kernel(x_h, c_h, wq_h, wuk_h, wuv_h, wo_h, bk_h, bv_h, sk_h, h_h, d_h, gw_h,
            o_h,
            x_v, c_v, wq_raw, wuk_raw, wuv_raw, wo_v, bk_s, bv_s, h_s,
            x_p, c_p, wq_s, wkv_s, q_s, k_s, v_s, ctx_s, kv_s, y_s, u_s, ht_s, f_s, g_s, o_s,
            sk_v, d_v, gw_v,
            sem_c, sem_x, sem_f, sem_g, sem_wo, sem_h, sem_small, sem_o):
    def cp_c(b):
        return pltpu.make_async_copy(c_h.at[pl.ds(b * RC, RC)], c_v.at[pl.ds(b * RC, RC)], sem_c.at[b])

    def cp_x(b):
        return pltpu.make_async_copy(x_h.at[pl.ds(b * RC, RC)], x_v.at[pl.ds(b * RC, RC)], sem_x.at[b])

    def cp_wq0(b):
        rows = pl.ds(b * 256, 256)
        return pltpu.make_async_copy(wq_h.at[rows, 0], wq_raw.at[0, rows], sem_f.at[b])

    def cp_wuk0(b):
        rows = pl.ds(b * 128, 128)
        return pltpu.make_async_copy(wuk_h.at[rows, 0], wuk_raw.at[0, rows], sem_f.at[4 + b])

    def cp_wuv0(b):
        rows = pl.ds(b * 128, 128)
        return pltpu.make_async_copy(wuv_h.at[rows, 0], wuv_raw.at[0, rows], sem_f.at[8 + b])

    def cp_b0(src, dst, pad, b, sem0):
        cg = b // 2
        r0 = (b % 2) * 1024
        return pltpu.make_async_copy(src.at[pl.ds(r0, 1024), pl.ds(cg * 128, 128)],
                                     dst.at[cg, pl.ds(pad + r0, 1024)], sem_f.at[sem0 + b])

    def cp_bk0(b):
        return cp_b0(bk_h, bk_s, PADK, b, 12)

    def cp_bv0(b):
        return cp_b0(bv_h, bv_s, 0, b, 16)

    def cp_h(g):
        return pltpu.make_async_copy(h_h.at[pl.ds(2 * g, 2)], h_s.at[pl.ds(2 * g, 2)], sem_h.at[g])

    def cp_wkv(g):
        return [pltpu.make_async_copy(wuk_h.at[:, g], wuk_raw.at[g], sem_g.at[g * 8]),
                pltpu.make_async_copy(wuv_h.at[:, g], wuv_raw.at[g], sem_g.at[g * 8 + 1])]

    def cp_kvaux(g):
        cps = [pltpu.make_async_copy(wq_h.at[:, g], wq_raw.at[g], sem_g.at[g * 8 + 2])]
        for u in range(2):
            cg = 2 * g + u
            cols = pl.ds(cg * 128, 128)
            cps.append(pltpu.make_async_copy(bk_h.at[:, cols], bk_s.at[cg, pl.ds(PADK, S)],
                                             sem_g.at[g * 8 + 3 + u]))
            cps.append(pltpu.make_async_copy(bv_h.at[:, cols], bv_s.at[cg], sem_g.at[g * 8 + 5 + u]))
        return cps

    cp_wo = pltpu.make_async_copy(wo_h, wo_v, sem_wo.at[0])
    cp_small = [pltpu.make_async_copy(sk_h, sk_v, sem_small.at[0]),
                pltpu.make_async_copy(d_h, d_v, sem_small.at[1]),
                pltpu.make_async_copy(gw_h, gw_v, sem_small.at[2])]

    def cp_o(r):
        rows = pl.ds(r * FO, FO)
        return pltpu.make_async_copy(o_s.at[rows], o_h.at[rows], sem_o.at[r])

    def start_kv0(b):
        cp_wq0(b).start()
        cp_bk0(b).start()
        cp_bv0(b).start()

    def relayout_wkv_step(g, b, s, which):
        m0 = pl.multiple_of(b * 128 + s * 32, 32)
        src = wuk_raw if which == 0 else wuv_raw
        t = jnp.swapaxes(src[g, pl.ds(m0, 32)], 0, 1)
        prow = pl.ds(pl.multiple_of(b * 64 + s * 16, 16), 16)
        for hh in range(HG):
            c0 = hh * 256 + which * 128
            wkv_s[prow, c0:c0 + 128] = _pk(t[hh])

    def stage_c(bn, rb):
        c_p[rb * 64:(rb + 1) * 64, :] = _pk(c_v[pl.ds(pl.multiple_of(bn * RC + rb * 128, 128), 128), :])

    def stage_x(bn, rb):
        x_p[rb * 64:(rb + 1) * 64, :] = _pk(x_v[pl.ds(pl.multiple_of(bn * RC + rb * 128, 128), 128), :])

    cp_c(0).start()
    cp_small[0].start()
    for b in range(4):
        cp_wuk0(b).start()
        cp_wuv0(b).start()

    fm, gm = _dft_mats()
    for hf in range(2):
        f_s[hf] = _pk(fm[hf])
        g_s[hf] = _pk(gm[hf])
    bk_s[:, 0:PADK, :] = jnp.zeros((NCG, PADK, 128), BF16)

    start_kv0(0)
    cp_small[1].start()
    cp_small[2].start()

    for b in range(4):
        cp_wuk0(b).wait()
        cp_wuv0(b).wait()
        for s in range(4):
            relayout_wkv_step(0, b, s, 0)
            relayout_wkv_step(0, b, s, 1)

    cp_small[0].wait()
    cp_c(0).wait()
    for rb in range(RC // 128):
        stage_c(0, rb)

    def group_body(g, carry):
        @pl.when(g + 1 < NG)
        def _():
            for cp in cp_wkv(g + 1):
                cp.start()

        @pl.when(g == 1)
        def _():
            cp_wo.start()

        @pl.when(g > 0)
        def _():
            for cp in cp_kvaux(g):
                cp.wait()

        def kv_body(b, c2):
            p = g * 4 + b

            def dma_g0():
                @pl.when(b > 0)
                def _():
                    cp_c(b).wait()
                    for rb in range(RC // 128):
                        stage_c(b, rb)
                cp_wq0(b).wait()
                cp_bk0(b).wait()
                cp_bv0(b).wait()

                @pl.when(b + 1 < NRC)
                def _():
                    cp_c(b + 1).start()
                    start_kv0(b + 1)

                @pl.when(b == 1)
                def _():
                    cp_x(0).start()
                    cp_x(1).start()
                    cp_h(0).start()

                @pl.when(b == 2)
                def _():
                    cp_x(2).start()
                    cp_x(3).start()
            _own_block((g == 0).astype(jnp.int32), dma_g0)
            bn = jnp.where(jnp.logical_and(g == 0, b + 1 < NRC), b, (b + 1) % NRC)

            def mm_piece(rb, hh):
                def run():
                    prow = pl.ds(pl.multiple_of(b * (RC // 2) + rb * 64, 64), 64)
                    kk = jnp.dot(_up(c_p[rb * 64:(rb + 1) * 64, :]), _up(wkv_s[:, hh * 256:(hh + 1) * 256]),
                                 preferred_element_type=F32)
                    k_s[hh, prow, :] = _pk((kk[:, 0:128] * QSCALE).astype(BF16))
                    v_s[hh, prow, :] = _pk(kk[:, 128:256].astype(BF16))
                return run

            def rq_step(s):
                def run():
                    m0 = pl.multiple_of(b * 256 + s * 32, 32)
                    t = jnp.swapaxes(wq_raw[g, pl.ds(m0, 32)], 0, 1)
                    prow = pl.ds(pl.multiple_of(b * 128 + s * 16, 16), 16)
                    for hh in range(HG):
                        wq_s[prow, hh * 128:(hh + 1) * 128] = _pk(t[hh])
                return run

            cg = p // 2
            rh = p % 2
            w = sk_v[:, pl.ds(pl.multiple_of(cg * 128, 128), 128)].astype(F32)

            def kvb_step(s):
                def run():
                    r0 = pl.multiple_of(rh * 1024 + s * 64, 64)
                    kw = bk_s[cg, pl.ds(r0, 64 + PADK), :].astype(F32)
                    acc = kw[PADK:] * w[0:1]
                    for j in range(1, 4):
                        acc = acc + kw[PADK - j:PADK - j + 64] * w[j:j + 1]
                    kvv = acc * bv_s[cg, pl.ds(r0, 64), :].astype(F32)
                    kv_s[cg, pl.ds(pl.multiple_of(rh * 512 + s * 32, 32), 32), :] = _pk(kvv.astype(BF16))
                return run

            aux = []
            for s in range(8):
                aux += [rq_step(s), kvb_step(2 * s), kvb_step(2 * s + 1)]
            k = 0
            done = 0
            for rb in range(RC // 128):
                for hh in range(HG):
                    mm_piece(rb, hh)()
                    k += 1
                    tgt = min(len(aux), (len(aux) * k) // 30)
                    while done < tgt:
                        aux[done]()
                        done += 1
                stage_c(bn, rb)
            return c2

        lax.fori_loop(0, NRC, kv_body, 0)

        def q_body(b, c2):
            bn = (b + 1) % NRC
            p = g * 4 + b
            cg = p // 2
            hf = p % 2

            def waits():
                @pl.when(jnp.logical_and(g == 0, b + 1 < NRC))
                def _():
                    cp_x(b + 1).wait()

                @pl.when(jnp.logical_and(g + 1 < NG, b == 0))
                def _():
                    for cp in cp_wkv(g + 1):
                        cp.wait()
            _own_block(jnp.logical_or(g == 0, b == 0).astype(jnp.int32), waits)

            gn = jnp.minimum(g + 1, NG - 1)
            fh = _up(f_s[hf])
            gh = _up(g_s[hf])
            st = {}

            def q_piece(rb, hh):
                def run():
                    prow = pl.ds(pl.multiple_of(b * (RC // 2) + rb * 64, 64), 64)
                    qq = jnp.dot(_up(x_p[rb * 64:(rb + 1) * 64, :]), _up(wq_s[:, hh * 128:(hh + 1) * 128]),
                                 preferred_element_type=F32)
                    q_s[hh, prow, :] = _pk(qq.astype(BF16))
                return run

            def u_piece(q):
                def run():
                    ucat = jnp.concatenate(
                        [_up(kv_s[cg, i * 64:(i + 1) * 64, :]) for i in range(4 * q, 4 * q + 4)], axis=1)
                    u_s[:, q * 512:(q + 1) * 512] = jnp.dot(fh, ucat, preferred_element_type=F32)
                return run

            def h_piece(q):
                def run():
                    hcat = jnp.concatenate(
                        [h_s[cg, :, m * CB:(m + 1) * CB] for m in range(4 * q, 4 * q + 4)], axis=0)
                    st["hh", q] = lax.dot_general(fh, hcat, NT, preferred_element_type=F32)
                return run

            sgn = jnp.where((lax.broadcasted_iota(jnp.int32, (64, 128), 0) & 1) == 0,
                            1.0, -1.0).astype(F32)

            def t_step(m):
                def run():
                    cur = st["hh", m // 4][:, (m % 4) * CB:(m % 4 + 1) * CB]
                    tr = sgn * cur[64:128]
                    ti = sgn * cur[0:64]
                    if m > 0:
                        prv = st["hh", (m - 1) // 4][:, ((m - 1) % 4) * CB:((m - 1) % 4 + 1) * CB]
                        tr = prv[0:64] + tr
                        ti = prv[64:128] - ti
                    else:
                        ti = -ti
                    ht_s[0:64, m * CB:(m + 1) * CB] = tr
                    ht_s[64:128, m * CB:(m + 1) * CB] = ti
                return run

            RB = 32

            def p_step(i, rb, m):
                def run():
                    a0 = (i - m) * CB
                    b0 = m * CB
                    ur = u_s[rb:rb + RB, a0:a0 + CB]
                    ui = u_s[64 + rb:64 + rb + RB, a0:a0 + CB]
                    hr = ht_s[rb:rb + RB, b0:b0 + CB]
                    hi = ht_s[64 + rb:64 + rb + RB, b0:b0 + CB]
                    pr = ur * hr - ui * hi
                    pi = ur * hi + ui * hr
                    if m > 0:
                        pr = st["yr"] + pr
                        pi = st["yi"] + pi
                    st["yr"], st["yi"] = pr, pi
                    if m == i:
                        st["Y", i, rb] = (pr.astype(BF16), pi.astype(BF16))
                return run

            def i_piece(q):
                def run():
                    blocks = []
                    for i in range(4 * q, 4 * q + 4):
                        parts = [st.pop(("Y", i, rb)) for rb in range(0, 64, RB)]
                        blocks.append(jnp.concatenate([t[0] for t in parts] + [t[1] for t in parts], axis=0))
                    st["yo", q] = jnp.dot(gh, jnp.concatenate(blocks, axis=1), preferred_element_type=F32)
                return run

            def y_step(i):
                def run():
                    yo = st["yo", i // 4][:, (i % 4) * CB:(i % 4 + 1) * CB]
                    old = jnp.where(hf == 0, 0.0, y_s[cg, i * CB:(i + 1) * CB, :])
                    y_s[cg, i * CB:(i + 1) * CB, :] = old + yo
                return run

            rsteps = [(lambda s=s, wh=wh: relayout_wkv_step(gn, b, s, wh)) for s in range(4) for wh in range(2)]
            for q in range(4):
                u_piece(q)()
            for q in range(4):
                h_piece(q)()
            qp = [q_piece(rb, hh) for rb in range(RC // 128) for hh in range(HG)]
            aux = [t_step(m) for m in range(NCB)]
            psteps = [(i, rb, m) for i in range(NCB) for rb in range(0, 64, RB) for m in range(i + 1)]
            NQ1 = 31
            per = len(psteps) / float(NQ1 - 1)
            done = 0
            pend_i = [0, 1, 2, 3]
            pend_y = []
            for k in range(len(qp)):
                qp[k]()
                if k % HG == HG - 1:
                    stage_x(bn, k // HG)
                if k == 0:
                    for a in aux:
                        a()
                    continue
                while pend_i and done >= 2 * sum(range(1, 4 * pend_i[0] + 5)) + (20 if pend_i[0] < 3 else 0):
                    q = pend_i.pop(0)
                    i_piece(q)()
                    pend_y += list(range(4 * q, 4 * q + 4))
                    break
                tgt = min(len(psteps), int(round(per * k)))
                while done < tgt:
                    p_step(*psteps[done])()
                    done += 1
                if k >= 1 and rsteps:
                    rsteps.pop(0)()
                ny = 1 if pend_i else 2
                for _ in range(ny):
                    if pend_y:
                        y_step(pend_y.pop(0))()
            assert not pend_i and not rsteps
            while pend_y:
                y_step(pend_y.pop(0))()
            return c2

        @pl.when(g + 1 < NG)
        def _():
            for cp in cp_kvaux(g + 1):
                cp.start()
            cp_h(g + 1).start()

        cp_h(g).wait()

        @pl.when(g == 0)
        def _():
            cp_x(0).wait()
            for rb in range(RC // 128):
                stage_x(0, rb)

        lax.fori_loop(0, NRC, q_body, 0)

        mask = (lax.broadcasted_iota(jnp.int32, (BQ, BQ), 1)
                <= lax.broadcasted_iota(jnp.int32, (BQ, BQ), 0))
        HB = BQ // 2

        def attn_body(t, c2):
            def qk(hh, i, z):
                q = q_s[hh, i * HB:(i + 1) * HB, :]
                if z is not None:
                    q = jnp.concatenate([q[0:8] + z, q[8:]], axis=0)
                return lax.dot_general(_up(q), _up(k_s[hh, 0:(i + 1) * HB, :]), NT,
                                       preferred_element_type=F32)

            def sm(i, s):
                L = (i + 1) * BQ
                sd = jnp.where(mask, s[:, L - BQ:], NEG)
                s = jnp.concatenate([s[:, :L - BQ], sd], axis=1) if i > 0 else sd
                m = jnp.max(s, axis=1, keepdims=True)
                p = jnp.exp2(s - m)
                l = jnp.sum(p, axis=1, keepdims=True)
                return p.astype(BF16), l

            def pv(hh, i, p):
                return jnp.dot(p, _up(v_s[hh, 0:(i + 1) * HB, :]), preferred_element_type=F32)

            def fin(hh, i, ctx, l):
                r = pl.reciprocal(l, approx=True)
                r = r * (2.0 - l * r)
                o = _pk((ctx * r).astype(BF16))
                ctx_s[g * HG + hh, i * HB:(i + 1) * HB, :] = o
                a = o[0:8]
                for kk in range(1, 8):
                    a = a | o[8 * kk:8 * kk + 8]
                return (a & 1) >> 1

            order = []
            for i in range(NBQ // 2):
                big, small = NBQ // 2 + i, (i + NBQ // 4) % (NBQ // 2)
                for u in range(0, AH, 2):
                    ha, hb = AH * t + u, AH * t + u + 1
                    order += [(ha, big), (hb, big), (hb, small), (ha, small)]
            n = len(order)
            lag = 3
            ss, cs, zs = {}, {}, {}
            ss[0] = qk(*order[0], None)
            for j in range(n + lag):
                if j + 1 < n:
                    ss[j + 1] = qk(*order[j + 1], zs.pop(j + 1, None))
                if j < n:
                    p, l = sm(order[j][1], ss.pop(j))
                    cs[j] = (pv(*order[j], p), l)
                if 0 <= j - lag < n:
                    zs[j + 2] = fin(*order[j - lag], *cs.pop(j - lag))
            return c2

        lax.fori_loop(0, HG // AH, attn_body, 0)
        return carry

    lax.fori_loop(0, NG, group_body, 0)

    cp_wo.wait()
    cp_small[1].wait()
    cp_small[2].wait()

    def out_body(r, carry):
        rows = pl.ds(pl.multiple_of(r * FO, FO), FO)
        prow = pl.ds(pl.multiple_of(r * (FO // 2), FO // 2), FO // 2)
        ctx = jnp.concatenate([_up(ctx_s[hh, prow, :]) for hh in range(H)], axis=1)
        a = jnp.dot(ctx, wo_v[...], preferred_element_type=F32)
        xf = x_v[rows, :].astype(F32)
        gw = gw_v[...].astype(F32)[None, :]
        gate = jax.nn.sigmoid(jnp.sum(xf * gw, axis=1, keepdims=True))
        dd = d_v[...].astype(F32)[None, :]
        for cg in range(NCG):
            cols = slice(cg * 128, (cg + 1) * 128)
            yb = y_s[cg, rows, :] + _up(kv_s[cg, prow, :]).astype(F32) * dd[:, cols]
            o_s[rows, cols] = (gate * a[:, cols] + (1.0 - gate) * (xf[:, cols] * yb)).astype(BF16)
        cp_o(r).start()
        return carry

    lax.fori_loop(0, S // FO, out_body, 0)
    for r in range(S // FO):
        cp_o(r).wait()


@jax.jit
def pallas_gated_mix__compressed_kv_cla__ssm_conv_h3__prompt_kernel(
    A_x: jax.Array,
    A_c_kv: jax.Array,
    A_w_q: jax.Array,
    A_w_uk: jax.Array,
    A_w_uv: jax.Array,
    A_w_o: jax.Array,
    B_q: jax.Array,
    B_k: jax.Array,
    B_v: jax.Array,
    B_shift_k: jax.Array,
    B_ssm_k: jax.Array,
    B_ssm_D: jax.Array,
    gate_w: jax.Array,
):
    del B_q
    x = A_x.reshape(S, M)
    c = A_c_kv.reshape(S, DC)
    wq = A_w_q.reshape(M, NG, HG, D)
    wuk = A_w_uk.reshape(DC, NG, HG, D)
    wuv = A_w_uv.reshape(DC, NG, HG, D)
    wo = A_w_o.reshape(H * D, M)
    bk = B_k.reshape(S, M)
    bv = B_v.reshape(S, M)
    skt = B_shift_k.T
    hk = B_ssm_k.reshape(NCG, 128, S)

    dma = pltpu.SemaphoreType.DMA
    scratch = [
        pltpu.VMEM((S, M), BF16),
        pltpu.VMEM((S, DC), BF16),
        pltpu.VMEM((NG, M, HG, D), BF16),
        pltpu.VMEM((NG, DC, HG, D), BF16),
        pltpu.VMEM((NG, DC, HG, D), BF16),
        pltpu.VMEM((H * D, M), BF16),
        pltpu.VMEM((NCG, PADK + S, 128), BF16),
        pltpu.VMEM((NCG, S, 128), BF16),
        pltpu.VMEM((NCG, 128, S), BF16),
        pltpu.VMEM((RC // 2, M), U32),
        pltpu.VMEM((RC // 2, DC), U32),
        pltpu.VMEM((M // 2, HG * D), U32),
        pltpu.VMEM((DC // 2, 2 * HG * D), U32),
        pltpu.VMEM((HG, S // 2, D), U32),
        pltpu.VMEM((HG, S // 2, D), U32),
        pltpu.VMEM((HG, S // 2, D), U32),
        pltpu.VMEM((H, S // 2, D), U32),
        pltpu.VMEM((NCG, S // 2, 128), U32),
        pltpu.VMEM((NCG, S, 128), F32),
        pltpu.VMEM((128, S), F32),
        pltpu.VMEM((128, S), F32),
        pltpu.VMEM((2, 64, 128), U32),
        pltpu.VMEM((2, 64, 128), U32),
        pltpu.VMEM((S, M), BF16),
        pltpu.VMEM((4, M), BF16),
        pltpu.VMEM((M,), BF16),
        pltpu.VMEM((M,), BF16),
        dma((4,)), dma((4,)), dma((20,)), dma((NG * 8,)), dma((1,)), dma((NG,)), dma((3,)),
        dma((S // FO,)),
    ]
    out = pl.pallas_call(
        _kernel,
        out_shape=jax.ShapeDtypeStruct((S, M), BF16),
        in_specs=[pl.BlockSpec(memory_space=pl.ANY)] * 12,
        out_specs=pl.BlockSpec(memory_space=pl.ANY),
        scratch_shapes=scratch,
        compiler_params=pltpu.CompilerParams(vmem_limit_bytes=120 * 1024 * 1024),
    )(x, c, wq, wuk, wuv, wo, bk, bv, skt, hk, B_ssm_D, gate_w)
    return out.reshape(1, S, M)
```

```python
import math

import jax
import jax.numpy as jnp
from jax import lax
import jax.experimental.pallas as pl
import jax.experimental.pallas.tpu as pltpu

F32 = jnp.float32
BF16 = jnp.bfloat16

S = 2048
M = 1024
H = 32
D = 128
DC = 512
HG = 8
NG = H // HG
RC = 512
NRC = S // RC
BQ = 128
NBQ = S // BQ
AH = 2
CB = 128
NCB = S // CB
NCG = M // 128
FO = 256
PADK = 16
NEG = -1e9
NT = (((1,), (1,)), ((), ()))
QSCALE = (D ** -0.5) * math.log2(math.e)


def _dft_mats():
    shp = (2, 128, 128)
    hf = lax.broadcasted_iota(jnp.int32, shp, 0)
    r = lax.broadcasted_iota(jnp.int32, shp, 1)
    j = lax.broadcasted_iota(jnp.int32, shp, 2)
    f = hf * 64 + (r & 63)
    k = ((2 * f + 1) * j + jnp.where(r >= 64, 128, 0)) & 511
    fm = jnp.cos(k.astype(F32) * (2 * math.pi / 512))
    ff = hf * 64 + (j & 63)
    k2 = ((2 * ff + 1) * (r + 128) + jnp.where(j >= 64, 128, 0)) & 511
    gm = jnp.cos(k2.astype(F32) * (2 * math.pi / 512)) * (1.0 / 128)
    return fm.astype(BF16), gm.astype(BF16)


U32 = jnp.uint32


def _pk(v):
    return pltpu.bitcast(v, U32)


def _up(v):
    return pltpu.bitcast(v, BF16)


def _own_block(trips, fn):
    def body(_, c):
        fn()
        return c
    lax.fori_loop(0, trips, body, 0)


def _spread(pieces, aux):
    n = len(pieces)
    done = 0
    for k, piece in enumerate(pieces):
        piece()
        tgt = (len(aux) * (k + 1)) // n
        while done < tgt:
            aux[done]()
            done += 1


def _kernel(x_h, c_h, wq_h, wuk_h, wuv_h, wo_h, bk_h, bv_h, sk_h, h_h, d_h, gw_h,
            o_h,
            x_v, c_v, wq_raw, wuk_raw, wuv_raw, wo_v, bk_s, bv_s, h_s,
            x_p, c_p, wq_s, wkv_s, q_s, k_s, v_s, ctx_s, kv_s, y_s, u_s, ht_s, f_s, g_s, o_s,
            sk_v, d_v, gw_v,
            sem_c, sem_x, sem_f, sem_g, sem_wo, sem_h, sem_small, sem_o):
    def cp_c(b):
        return pltpu.make_async_copy(c_h.at[pl.ds(b * RC, RC)], c_v.at[pl.ds(b * RC, RC)], sem_c.at[b])

    def cp_x(b):
        return pltpu.make_async_copy(x_h.at[pl.ds(b * RC, RC)], x_v.at[pl.ds(b * RC, RC)], sem_x.at[b])

    def cp_wq0(b):
        rows = pl.ds(b * 256, 256)
        return pltpu.make_async_copy(wq_h.at[rows, 0], wq_raw.at[0, rows], sem_f.at[b])

    def cp_wuk0(b):
        rows = pl.ds(b * 128, 128)
        return pltpu.make_async_copy(wuk_h.at[rows, 0], wuk_raw.at[0, rows], sem_f.at[4 + b])

    def cp_wuv0(b):
        rows = pl.ds(b * 128, 128)
        return pltpu.make_async_copy(wuv_h.at[rows, 0], wuv_raw.at[0, rows], sem_f.at[8 + b])

    def cp_b0(src, dst, pad, b, sem0):
        cg = b // 2
        r0 = (b % 2) * 1024
        return pltpu.make_async_copy(src.at[pl.ds(r0, 1024), pl.ds(cg * 128, 128)],
                                     dst.at[cg, pl.ds(pad + r0, 1024)], sem_f.at[sem0 + b])

    def cp_bk0(b):
        return cp_b0(bk_h, bk_s, PADK, b, 12)

    def cp_bv0(b):
        return cp_b0(bv_h, bv_s, 0, b, 16)

    def cp_h(g):
        return pltpu.make_async_copy(h_h.at[pl.ds(2 * g, 2)], h_s.at[pl.ds(2 * g, 2)], sem_h.at[g])

    def cp_wkv(g):
        return [pltpu.make_async_copy(wuk_h.at[:, g], wuk_raw.at[g], sem_g.at[g * 8]),
                pltpu.make_async_copy(wuv_h.at[:, g], wuv_raw.at[g], sem_g.at[g * 8 + 1])]

    def cp_kvaux(g):
        cps = [pltpu.make_async_copy(wq_h.at[:, g], wq_raw.at[g], sem_g.at[g * 8 + 2])]
        for u in range(2):
            cg = 2 * g + u
            cols = pl.ds(cg * 128, 128)
            cps.append(pltpu.make_async_copy(bk_h.at[:, cols], bk_s.at[cg, pl.ds(PADK, S)],
                                             sem_g.at[g * 8 + 3 + u]))
            cps.append(pltpu.make_async_copy(bv_h.at[:, cols], bv_s.at[cg], sem_g.at[g * 8 + 5 + u]))
        return cps

    cp_wo = pltpu.make_async_copy(wo_h, wo_v, sem_wo.at[0])
    cp_small = [pltpu.make_async_copy(sk_h, sk_v, sem_small.at[0]),
                pltpu.make_async_copy(d_h, d_v, sem_small.at[1]),
                pltpu.make_async_copy(gw_h, gw_v, sem_small.at[2])]

    def cp_o(r):
        rows = pl.ds(r * FO, FO)
        return pltpu.make_async_copy(o_s.at[rows], o_h.at[rows], sem_o.at[r])

    def start_kv0(b):
        cp_wq0(b).start()
        cp_bk0(b).start()
        cp_bv0(b).start()

    def relayout_wkv_step(g, b, s, which):
        m0 = pl.multiple_of(b * 128 + s * 32, 32)
        src = wuk_raw if which == 0 else wuv_raw
        t = jnp.swapaxes(src[g, pl.ds(m0, 32)], 0, 1)
        prow = pl.ds(pl.multiple_of(b * 64 + s * 16, 16), 16)
        for hh in range(HG):
            c0 = hh * 256 + which * 128
            wkv_s[prow, c0:c0 + 128] = _pk(t[hh])

    def stage_c(bn, rb):
        c_p[rb * 64:(rb + 1) * 64, :] = _pk(c_v[pl.ds(pl.multiple_of(bn * RC + rb * 128, 128), 128), :])

    def stage_x(bn, rb):
        x_p[rb * 64:(rb + 1) * 64, :] = _pk(x_v[pl.ds(pl.multiple_of(bn * RC + rb * 128, 128), 128), :])

    cp_c(0).start()
    cp_small[0].start()
    for b in range(4):
        cp_wuk0(b).start()
        cp_wuv0(b).start()

    fm, gm = _dft_mats()
    for hf in range(2):
        f_s[hf] = _pk(fm[hf])
        g_s[hf] = _pk(gm[hf])
    bk_s[:, 0:PADK, :] = jnp.zeros((NCG, PADK, 128), BF16)

    start_kv0(0)
    cp_small[1].start()
    cp_small[2].start()

    for b in range(4):
        cp_wuk0(b).wait()
        cp_wuv0(b).wait()
        for s in range(4):
            relayout_wkv_step(0, b, s, 0)
            relayout_wkv_step(0, b, s, 1)

    cp_small[0].wait()
    cp_c(0).wait()
    for rb in range(RC // 128):
        stage_c(0, rb)

    def group_body(g, carry):
        @pl.when(g + 1 < NG)
        def _():
            for cp in cp_wkv(jnp.minimum(g + 1, NG - 1)):
                cp.start()

        @pl.when(g == 1)
        def _():
            cp_wo.start()

        @pl.when(g > 0)
        def _():
            for cp in cp_kvaux(g):
                cp.wait()

        def kv_body(b, c2):
            p = g * 4 + b

            def dma_g0():
                @pl.when(b > 0)
                def _():
                    cp_c(b).wait()
                    for rb in range(RC // 128):
                        stage_c(b, rb)
                cp_wq0(b).wait()
                cp_bk0(b).wait()
                cp_bv0(b).wait()

                @pl.when(b + 1 < NRC)
                def _():
                    cp_c(jnp.minimum(b + 1, NRC - 1)).start()
                    start_kv0(jnp.minimum(b + 1, NRC - 1))

                @pl.when(b == 1)
                def _():
                    cp_x(0).start()
                    cp_x(1).start()
                    cp_h(0).start()

                @pl.when(b == 2)
                def _():
                    cp_x(2).start()
                    cp_x(3).start()
            _own_block((g == 0).astype(jnp.int32), dma_g0)
            bn = jnp.where(jnp.logical_and(g == 0, b + 1 < NRC), b, (b + 1) % NRC)

            def mm_piece(rb, hh):
                def run():
                    prow = pl.ds(pl.multiple_of(b * (RC // 2) + rb * 64, 64), 64)
                    kk = jnp.dot(_up(c_p[rb * 64:(rb + 1) * 64, :]), _up(wkv_s[:, hh * 256:(hh + 1) * 256]),
                                 preferred_element_type=F32)
                    k_s[hh, prow, :] = _pk((kk[:, 0:128] * QSCALE).astype(BF16))
                    v_s[hh, prow, :] = _pk(kk[:, 128:256].astype(BF16))
                return run

            def rq_step(s):
                def run():
                    m0 = pl.multiple_of(b * 256 + s * 32, 32)
                    t = jnp.swapaxes(wq_raw[g, pl.ds(m0, 32)], 0, 1)
                    prow = pl.ds(pl.multiple_of(b * 128 + s * 16, 16), 16)
                    for hh in range(HG):
                        wq_s[prow, hh * 128:(hh + 1) * 128] = _pk(t[hh])
                return run

            cg = p // 2
            rh = p % 2
            w = sk_v[:, pl.ds(pl.multiple_of(cg * 128, 128), 128)].astype(F32)

            def kvb_step(s):
                def run():
                    r0 = pl.multiple_of(rh * 1024 + s * 64, 64)
                    kw = bk_s[cg, pl.ds(r0, 64 + PADK), :].astype(F32)
                    acc = kw[PADK:] * w[0:1]
                    for j in range(1, 4):
                        acc = acc + kw[PADK - j:PADK - j + 64] * w[j:j + 1]
                    kvv = acc * bv_s[cg, pl.ds(r0, 64), :].astype(F32)
                    kv_s[cg, pl.ds(pl.multiple_of(rh * 512 + s * 32, 32), 32), :] = _pk(kvv.astype(BF16))
                return run

            aux = []
            for s in range(8):
                aux += [rq_step(s), kvb_step(2 * s), kvb_step(2 * s + 1)]
            k = 0
            done = 0
            for rb in range(RC // 128):
                for hh in range(HG):
                    mm_piece(rb, hh)()
                    k += 1
                    tgt = min(len(aux), (len(aux) * k) // 30)
                    while done < tgt:
                        aux[done]()
                        done += 1
                stage_c(bn, rb)
            return c2

        lax.fori_loop(0, NRC, kv_body, 0)

        def q_body(b, c2):
            bn = (b + 1) % NRC
            p = g * 4 + b
            cg = p // 2
            hf = p % 2
            gn = jnp.minimum(g + 1, NG - 1)

            def waits():
                @pl.when(jnp.logical_and(g == 0, b + 1 < NRC))
                def _():
                    cp_x(jnp.minimum(b + 1, NRC - 1)).wait()

                @pl.when(jnp.logical_and(g + 1 < NG, b == 0))
                def _():
                    for cp in cp_wkv(gn):
                        cp.wait()
            _own_block(jnp.logical_or(g == 0, b == 0).astype(jnp.int32), waits)

            fh = _up(f_s[hf])
            gh = _up(g_s[hf])
            st = {}

            def q_piece(rb, hh):
                def run():
                    prow = pl.ds(pl.multiple_of(b * (RC // 2) + rb * 64, 64), 64)
                    qq = jnp.dot(_up(x_p[rb * 64:(rb + 1) * 64, :]), _up(wq_s[:, hh * 128:(hh + 1) * 128]),
                                 preferred_element_type=F32)
                    q_s[hh, prow, :] = _pk(qq.astype(BF16))
                return run

            def u_piece(q):
                def run():
                    ucat = jnp.concatenate(
                        [_up(kv_s[cg, i * 64:(i + 1) * 64, :]) for i in range(4 * q, 4 * q + 4)], axis=1)
                    u_s[:, q * 512:(q + 1) * 512] = jnp.dot(fh, ucat, preferred_element_type=F32)
                return run

            def h_piece(q):
                def run():
                    hcat = jnp.concatenate(
                        [h_s[cg, :, m * CB:(m + 1) * CB] for m in range(4 * q, 4 * q + 4)], axis=0)
                    st["hh", q] = lax.dot_general(fh, hcat, NT, preferred_element_type=F32)
                return run

            sgn = jnp.where((lax.broadcasted_iota(jnp.int32, (64, 128), 0) & 1) == 0,
                            1.0, -1.0).astype(F32)

            def t_step(m):
                def run():
                    cur = st["hh", m // 4][:, (m % 4) * CB:(m % 4 + 1) * CB]
                    tr = sgn * cur[64:128]
                    ti = sgn * cur[0:64]
                    if m > 0:
                        prv = st["hh", (m - 1) // 4][:, ((m - 1) % 4) * CB:((m - 1) % 4 + 1) * CB]
                        tr = prv[0:64] + tr
                        ti = prv[64:128] - ti
                    else:
                        ti = -ti
                    ht_s[0:64, m * CB:(m + 1) * CB] = tr
                    ht_s[64:128, m * CB:(m + 1) * CB] = ti
                return run

            RB = 32

            def p_step(i, rb, m):
                def run():
                    a0 = (i - m) * CB
                    b0 = m * CB
                    ur = u_s[rb:rb + RB, a0:a0 + CB]
                    ui = u_s[64 + rb:64 + rb + RB, a0:a0 + CB]
                    hr = ht_s[rb:rb + RB, b0:b0 + CB]
                    hi = ht_s[64 + rb:64 + rb + RB, b0:b0 + CB]
                    pr = ur * hr - ui * hi
                    pi = ur * hi + ui * hr
                    if m > 0:
                        pr = st["yr"] + pr
                        pi = st["yi"] + pi
                    st["yr"], st["yi"] = pr, pi
                    if m == i:
                        st["Y", i, rb] = (pr.astype(BF16), pi.astype(BF16))
                return run

            def i_piece(q):
                def run():
                    blocks = []
                    for i in range(4 * q, 4 * q + 4):
                        parts = [st.pop(("Y", i, rb)) for rb in range(0, 64, RB)]
                        blocks.append(jnp.concatenate([t[0] for t in parts] + [t[1] for t in parts], axis=0))
                    st["yo", q] = jnp.dot(gh, jnp.concatenate(blocks, axis=1), preferred_element_type=F32)
                return run

            def y_step(i):
                def run():
                    yo = st["yo", i // 4][:, (i % 4) * CB:(i % 4 + 1) * CB]
                    old = jnp.where(hf == 0, 0.0, y_s[cg, i * CB:(i + 1) * CB, :])
                    y_s[cg, i * CB:(i + 1) * CB, :] = old + yo
                return run

            rsteps = [(lambda s=s, wh=wh: relayout_wkv_step(gn, b, s, wh)) for s in range(4) for wh in range(2)]
            for q in range(4):
                u_piece(q)()
            for q in range(4):
                h_piece(q)()
            qp = [q_piece(rb, hh) for rb in range(RC // 128) for hh in range(HG)]
            aux = [t_step(m) for m in range(NCB)]
            psteps = [(i, rb, m) for i in range(NCB) for rb in range(0, 64, RB) for m in range(i + 1)]
            NQ1 = 31
            per = len(psteps) / float(NQ1 - 1)
            done = 0
            pend_i = [0, 1, 2, 3]
            pend_y = []
            for k in range(len(qp)):
                qp[k]()
                if k % HG == HG - 1:
                    stage_x(bn, k // HG)
                if k == 0:
                    for a in aux:
                        a()
                    continue
                while pend_i and done >= 2 * sum(range(1, 4 * pend_i[0] + 5)) + (20 if pend_i[0] < 3 else 0):
                    q = pend_i.pop(0)
                    i_piece(q)()
                    pend_y += list(range(4 * q, 4 * q + 4))
                    break
                tgt = min(len(psteps), int(round(per * k)))
                while done < tgt:
                    p_step(*psteps[done])()
                    done += 1
                if k >= 1 and rsteps:
                    rsteps.pop(0)()
                ny = 1 if pend_i else 2
                for _ in range(ny):
                    if pend_y:
                        y_step(pend_y.pop(0))()
            assert not pend_i and not rsteps
            while pend_y:
                y_step(pend_y.pop(0))()
            return c2

        @pl.when(g + 1 < NG)
        def _():
            for cp in cp_kvaux(jnp.minimum(g + 1, NG - 1)):
                cp.start()
            cp_h(jnp.minimum(g + 1, NG - 1)).start()

        cp_h(g).wait()

        @pl.when(g == 0)
        def _():
            cp_x(0).wait()
            for rb in range(RC // 128):
                stage_x(0, rb)

        lax.fori_loop(0, NRC, q_body, 0)

        mask = (lax.broadcasted_iota(jnp.int32, (BQ, BQ), 1)
                <= lax.broadcasted_iota(jnp.int32, (BQ, BQ), 0))
        HB = BQ // 2

        def attn_body(t, c2):
            def qk(hh, i, z):
                q = q_s[hh, i * HB:(i + 1) * HB, :]
                if z is not None:
                    q = jnp.concatenate([q[0:8] + z, q[8:]], axis=0)
                return lax.dot_general(_up(q), _up(k_s[hh, 0:(i + 1) * HB, :]), NT,
                                       preferred_element_type=F32)

            def sm(i, s):
                L = (i + 1) * BQ
                sd = jnp.where(mask, s[:, L - BQ:], NEG)
                s = jnp.concatenate([s[:, :L - BQ], sd], axis=1) if i > 0 else sd
                m = jnp.max(s, axis=1, keepdims=True)
                p = jnp.exp2(s - m)
                l = jnp.sum(p, axis=1, keepdims=True)
                return p.astype(BF16), l

            def pv(hh, i, p):
                return jnp.dot(p, _up(v_s[hh, 0:(i + 1) * HB, :]), preferred_element_type=F32)

            def fin(hh, i, ctx, l):
                r = pl.reciprocal(l, approx=True)
                r = r * (2.0 - l * r)
                o = _pk((ctx * r).astype(BF16))
                ctx_s[g * HG + hh, i * HB:(i + 1) * HB, :] = o
                a = o[0:8]
                for kk in range(1, 8):
                    a = a | o[8 * kk:8 * kk + 8]
                return (a & 1) >> 1

            order = []
            for i in range(NBQ // 2):
                big, small = NBQ // 2 + i, (i + NBQ // 4) % (NBQ // 2)
                for u in range(0, AH, 2):
                    ha, hb = AH * t + u, AH * t + u + 1
                    order += [(ha, big), (hb, big), (hb, small), (ha, small)]
            n = len(order)
            lag = 3
            ss, cs, zs = {}, {}, {}
            ss[0] = qk(*order[0], None)
            for j in range(n + lag):
                if j + 1 < n:
                    ss[j + 1] = qk(*order[j + 1], zs.pop(j + 1, None))
                if j < n:
                    p, l = sm(order[j][1], ss.pop(j))
                    cs[j] = (pv(*order[j], p), l)
                if 0 <= j - lag < n:
                    zs[j + 2] = fin(*order[j - lag], *cs.pop(j - lag))
            return c2

        lax.fori_loop(0, HG // AH, attn_body, 0)
        return carry

    lax.fori_loop(0, NG, group_body, 0)

    cp_wo.wait()
    cp_small[1].wait()
    cp_small[2].wait()

    def out_body(r, carry):
        rows = pl.ds(pl.multiple_of(r * FO, FO), FO)
        prow = pl.ds(pl.multiple_of(r * (FO // 2), FO // 2), FO // 2)
        ctx = jnp.concatenate([_up(ctx_s[hh, prow, :]) for hh in range(H)], axis=1)
        a = jnp.dot(ctx, wo_v[...], preferred_element_type=F32)
        xf = x_v[rows, :].astype(F32)
        gw = gw_v[...].astype(F32)[None, :]
        gate = jax.nn.sigmoid(jnp.sum(xf * gw, axis=1, keepdims=True))
        dd = d_v[...].astype(F32)[None, :]
        for cg in range(NCG):
            cols = slice(cg * 128, (cg + 1) * 128)
            yb = y_s[cg, rows, :] + _up(kv_s[cg, prow, :]).astype(F32) * dd[:, cols]
            o_s[rows, cols] = (gate * a[:, cols] + (1.0 - gate) * (xf[:, cols] * yb)).astype(BF16)
        cp_o(r).start()
        return carry

    lax.fori_loop(0, S // FO, out_body, 0)
    for r in range(S // FO):
        cp_o(r).wait()


@jax.jit
def pallas_gated_mix__compressed_kv_cla__ssm_conv_h3__prompt_kernel(
    A_x: jax.Array,
    A_c_kv: jax.Array,
    A_w_q: jax.Array,
    A_w_uk: jax.Array,
    A_w_uv: jax.Array,
    A_w_o: jax.Array,
    B_q: jax.Array,
    B_k: jax.Array,
    B_v: jax.Array,
    B_shift_k: jax.Array,
    B_ssm_k: jax.Array,
    B_ssm_D: jax.Array,
    gate_w: jax.Array,
):
    del B_q
    x = A_x.reshape(S, M)
    c = A_c_kv.reshape(S, DC)
    wq = A_w_q.reshape(M, NG, HG, D)
    wuk = A_w_uk.reshape(DC, NG, HG, D)
    wuv = A_w_uv.reshape(DC, NG, HG, D)
    wo = A_w_o.reshape(H * D, M)
    bk = B_k.reshape(S, M)
    bv = B_v.reshape(S, M)
    skt = B_shift_k.T
    hk = B_ssm_k.reshape(NCG, 128, S)

    dma = pltpu.SemaphoreType.DMA
    scratch = [
        pltpu.VMEM((S, M), BF16),
        pltpu.VMEM((S, DC), BF16),
        pltpu.VMEM((NG, M, HG, D), BF16),
        pltpu.VMEM((NG, DC, HG, D), BF16),
        pltpu.VMEM((NG, DC, HG, D), BF16),
        pltpu.VMEM((H * D, M), BF16),
        pltpu.VMEM((NCG, PADK + S, 128), BF16),
        pltpu.VMEM((NCG, S, 128), BF16),
        pltpu.VMEM((NCG, 128, S), BF16),
        pltpu.VMEM((RC // 2, M), U32),
        pltpu.VMEM((RC // 2, DC), U32),
        pltpu.VMEM((M // 2, HG * D), U32),
        pltpu.VMEM((DC // 2, 2 * HG * D), U32),
        pltpu.VMEM((HG, S // 2, D), U32),
        pltpu.VMEM((HG, S // 2, D), U32),
        pltpu.VMEM((HG, S // 2, D), U32),
        pltpu.VMEM((H, S // 2, D), U32),
        pltpu.VMEM((NCG, S // 2, 128), U32),
        pltpu.VMEM((NCG, S, 128), F32),
        pltpu.VMEM((128, S), F32),
        pltpu.VMEM((128, S), F32),
        pltpu.VMEM((2, 64, 128), U32),
        pltpu.VMEM((2, 64, 128), U32),
        pltpu.VMEM((S, M), BF16),
        pltpu.VMEM((4, M), BF16),
        pltpu.VMEM((M,), BF16),
        pltpu.VMEM((M,), BF16),
        dma((4,)), dma((4,)), dma((20,)), dma((NG * 8,)), dma((1,)), dma((NG,)), dma((3,)),
        dma((S // FO,)),
    ]
    out = pl.pallas_call(
        _kernel,
        out_shape=jax.ShapeDtypeStruct((S, M), BF16),
        in_specs=[pl.BlockSpec(memory_space=pl.ANY)] * 12,
        out_specs=pl.BlockSpec(memory_space=pl.ANY),
        scratch_shapes=scratch,
        compiler_params=pltpu.CompilerParams(vmem_limit_bytes=120 * 1024 * 1024),
    )(x, c, wq, wuk, wuv, wo, bk, bv, skt, hk, B_ssm_D, gate_w)
    return out.reshape(1, S, M)
```

```python
import math

import jax
import jax.numpy as jnp
from jax import lax
import jax.experimental.pallas as pl
import jax.experimental.pallas.tpu as pltpu

F32 = jnp.float32
BF16 = jnp.bfloat16
U32 = jnp.uint32

S = 2048
M = 1024
H = 32
D = 128
DC = 512
HG = 8
NG = H // HG
RC = 512
NRC = S // RC
BQ = 128
NBQ = S // BQ
AH = 2
CB = 128
NCB = S // CB
NCG = M // 128
FO = 256
PADK = 16
NEG = -1e9
NT = (((1,), (1,)), ((), ()))
QSCALE = (D ** -0.5) * math.log2(math.e)


def _dft_mats():
    shp = (2, 128, 128)
    hf = lax.broadcasted_iota(jnp.int32, shp, 0)
    r = lax.broadcasted_iota(jnp.int32, shp, 1)
    j = lax.broadcasted_iota(jnp.int32, shp, 2)
    f = hf * 64 + (r & 63)
    k = ((2 * f + 1) * j + jnp.where(r >= 64, 128, 0)) & 511
    fm = jnp.cos(k.astype(F32) * (2 * math.pi / 512))
    ff = hf * 64 + (j & 63)
    k2 = ((2 * ff + 1) * (r + 128) + jnp.where(j >= 64, 128, 0)) & 511
    gm = jnp.cos(k2.astype(F32) * (2 * math.pi / 512)) * (1.0 / 128)
    return fm.astype(BF16), gm.astype(BF16)


def _pk(v):
    return pltpu.bitcast(v, U32)


def _up(v):
    return pltpu.bitcast(v, BF16)


def _own_block(trips, fn):
    def body(_, c):
        fn()
        return c
    lax.fori_loop(0, trips, body, 0)


def _kernel(x_h, c_h, wq_h, wuk_h, wuv_h, wo_h, bk_h, bv_h, sk_h, h_h, d_h, gw_h,
            o_h,
            x_v, c_v, wq_raw, wuk_raw, wuv_raw, wo_v, bk_s, bv_s, h_s,
            x_p, c_p, wq_s, wkv_s, q_s, k_s, v_s, ctx_s, kv_s, y_s, u_s, ht_s, f_s, g_s, o_s,
            sk_v, d_v, gw_v,
            sem_c, sem_x, sem_f, sem_g, sem_wo, sem_h, sem_small, sem_o):
    def cp_c(b):
        return pltpu.make_async_copy(c_h.at[pl.ds(b * RC, RC)], c_v.at[pl.ds(b * RC, RC)], sem_c.at[b])

    def cp_x(b):
        return pltpu.make_async_copy(x_h.at[pl.ds(b * RC, RC)], x_v.at[pl.ds(b * RC, RC)], sem_x.at[b])

    def cp_wq0(b):
        rows = pl.ds(b * 256, 256)
        return pltpu.make_async_copy(wq_h.at[rows, 0], wq_raw.at[0, rows], sem_f.at[b])

    def cp_wuk0(b):
        rows = pl.ds(b * 128, 128)
        return pltpu.make_async_copy(wuk_h.at[rows, 0], wuk_raw.at[0, rows], sem_f.at[4 + b])

    def cp_wuv0(b):
        rows = pl.ds(b * 128, 128)
        return pltpu.make_async_copy(wuv_h.at[rows, 0], wuv_raw.at[0, rows], sem_f.at[8 + b])

    def cp_b0(src, dst, pad, b, sem0):
        cg = b // 2
        r0 = (b % 2) * 1024
        return pltpu.make_async_copy(src.at[pl.ds(r0, 1024), pl.ds(cg * 128, 128)],
                                     dst.at[cg, pl.ds(pad + r0, 1024)], sem_f.at[sem0 + b])

    def cp_bk0(b):
        return cp_b0(bk_h, bk_s, PADK, b, 12)

    def cp_bv0(b):
        return cp_b0(bv_h, bv_s, 0, b, 16)

    def cp_h(g):
        return pltpu.make_async_copy(h_h.at[pl.ds(2 * g, 2)], h_s.at[pl.ds(2 * g, 2)], sem_h.at[g])

    def cp_wkv(g):
        return [pltpu.make_async_copy(wuk_h.at[:, g], wuk_raw.at[g], sem_g.at[g * 8]),
                pltpu.make_async_copy(wuv_h.at[:, g], wuv_raw.at[g], sem_g.at[g * 8 + 1])]

    def cp_kvaux(g):
        cps = [pltpu.make_async_copy(wq_h.at[:, g], wq_raw.at[g], sem_g.at[g * 8 + 2])]
        for u in range(2):
            cg = 2 * g + u
            cols = pl.ds(cg * 128, 128)
            cps.append(pltpu.make_async_copy(bk_h.at[:, cols], bk_s.at[cg, pl.ds(PADK, S)],
                                             sem_g.at[g * 8 + 3 + u]))
            cps.append(pltpu.make_async_copy(bv_h.at[:, cols], bv_s.at[cg], sem_g.at[g * 8 + 5 + u]))
        return cps

    cp_wo = pltpu.make_async_copy(wo_h, wo_v, sem_wo.at[0])
    cp_small = [pltpu.make_async_copy(sk_h, sk_v, sem_small.at[0]),
                pltpu.make_async_copy(d_h, d_v, sem_small.at[1]),
                pltpu.make_async_copy(gw_h, gw_v, sem_small.at[2])]

    def cp_o(r):
        rows = pl.ds(r * FO, FO)
        return pltpu.make_async_copy(o_s.at[rows], o_h.at[rows], sem_o.at[r])

    def start_kv0(b):
        cp_wq0(b).start()
        cp_bk0(b).start()
        cp_bv0(b).start()

    def relayout_wkv_step(g, b, s, which):
        m0 = pl.multiple_of(b * 128 + s * 32, 32)
        src = wuk_raw if which == 0 else wuv_raw
        t = jnp.swapaxes(src[g, pl.ds(m0, 32)], 0, 1)
        prow = pl.ds(pl.multiple_of(b * 64 + s * 16, 16), 16)
        for hh in range(HG):
            c0 = hh * 256 + which * 128
            wkv_s[prow, c0:c0 + 128] = _pk(t[hh])

    def stage_c(bn, rb):
        c_p[rb * 64:(rb + 1) * 64, :] = _pk(c_v[pl.ds(pl.multiple_of(bn * RC + rb * 128, 128), 128), :])

    def stage_x(bn, rb):
        x_p[rb * 64:(rb + 1) * 64, :] = _pk(x_v[pl.ds(pl.multiple_of(bn * RC + rb * 128, 128), 128), :])

    cp_c(0).start()
    cp_small[0].start()
    for b in range(4):
        cp_wuk0(b).start()
        cp_wuv0(b).start()

    fm, gm = _dft_mats()
    for hf in range(2):
        f_s[hf] = _pk(fm[hf])
        g_s[hf] = _pk(gm[hf])
    bk_s[:, 0:PADK, :] = jnp.zeros((NCG, PADK, 128), BF16)

    start_kv0(0)
    cp_small[1].start()
    cp_small[2].start()

    for b in range(4):
        cp_wuk0(b).wait()
        cp_wuv0(b).wait()
        for s in range(4):
            relayout_wkv_step(0, b, s, 0)
            relayout_wkv_step(0, b, s, 1)

    cp_small[0].wait()
    cp_c(0).wait()
    for rb in range(RC // 128):
        stage_c(0, rb)

    def group_body(g, carry):
        @pl.when(g + 1 < NG)
        def _():
            for cp in cp_wkv(jnp.minimum(g + 1, NG - 1)):
                cp.start()

        @pl.when(g == 1)
        def _():
            cp_wo.start()

        @pl.when(g > 0)
        def _():
            for cp in cp_kvaux(g):
                cp.wait()

        def kv_body(b, c2):
            p = g * 4 + b

            def dma_g0():
                @pl.when(b > 0)
                def _():
                    cp_c(b).wait()
                    for rb in range(RC // 128):
                        stage_c(b, rb)
                cp_wq0(b).wait()
                cp_bk0(b).wait()
                cp_bv0(b).wait()

                @pl.when(b + 1 < NRC)
                def _():
                    cp_c(jnp.minimum(b + 1, NRC - 1)).start()
                    start_kv0(jnp.minimum(b + 1, NRC - 1))

                @pl.when(b == 1)
                def _():
                    cp_x(0).start()
                    cp_x(1).start()
                    cp_h(0).start()

                @pl.when(b == 2)
                def _():
                    cp_x(2).start()
                    cp_x(3).start()
            _own_block((g == 0).astype(jnp.int32), dma_g0)
            bn = jnp.where(jnp.logical_and(g == 0, b + 1 < NRC), b, (b + 1) % NRC)

            def mm_piece(rb, hh):
                def run():
                    prow = pl.ds(pl.multiple_of(b * (RC // 2) + rb * 64, 64), 64)
                    kk = jnp.dot(_up(c_p[rb * 64:(rb + 1) * 64, :]), _up(wkv_s[:, hh * 256:(hh + 1) * 256]),
                                 preferred_element_type=F32)
                    k_s[hh, prow, :] = _pk((kk[:, 0:128] * QSCALE).astype(BF16))
                    v_s[hh, prow, :] = _pk(kk[:, 128:256].astype(BF16))
                return run

            def rq_step(s):
                def run():
                    m0 = pl.multiple_of(b * 256 + s * 32, 32)
                    t = jnp.swapaxes(wq_raw[g, pl.ds(m0, 32)], 0, 1)
                    prow = pl.ds(pl.multiple_of(b * 128 + s * 16, 16), 16)
                    for hh in range(HG):
                        wq_s[prow, hh * 128:(hh + 1) * 128] = _pk(t[hh])
                return run

            cg = p // 2
            rh = p % 2
            w = sk_v[:, pl.ds(pl.multiple_of(cg * 128, 128), 128)].astype(F32)

            def kvb_step(s):
                def run():
                    r0 = pl.multiple_of(rh * 1024 + s * 64, 64)
                    kw = bk_s[cg, pl.ds(r0, 64 + PADK), :].astype(F32)
                    acc = kw[PADK:] * w[0:1]
                    for j in range(1, 4):
                        acc = acc + kw[PADK - j:PADK - j + 64] * w[j:j + 1]
                    kvv = acc * bv_s[cg, pl.ds(r0, 64), :].astype(F32)
                    kv_s[cg, pl.ds(pl.multiple_of(rh * 512 + s * 32, 32), 32), :] = _pk(kvv.astype(BF16))
                return run

            aux = []
            for s in range(8):
                aux += [rq_step(s), kvb_step(2 * s), kvb_step(2 * s + 1)]
            k = 0
            done = 0
            for rb in range(RC // 128):
                for hh in range(HG):
                    mm_piece(rb, hh)()
                    k += 1
                    tgt = min(len(aux), (len(aux) * k) // 30)
                    while done < tgt:
                        aux[done]()
                        done += 1
                stage_c(bn, rb)
            return c2

        lax.fori_loop(0, NRC, kv_body, 0)

        def q_body(b, c2):
            bn = (b + 1) % NRC
            p = g * 4 + b
            cg = p // 2
            hf = p % 2
            gn = jnp.minimum(g + 1, NG - 1)

            def waits():
                @pl.when(jnp.logical_and(g == 0, b + 1 < NRC))
                def _():
                    cp_x(jnp.minimum(b + 1, NRC - 1)).wait()

                @pl.when(jnp.logical_and(g + 1 < NG, b == 0))
                def _():
                    for cp in cp_wkv(gn):
                        cp.wait()
            _own_block(jnp.logical_or(g == 0, b == 0).astype(jnp.int32), waits)

            fh = _up(f_s[hf])
            gh = _up(g_s[hf])
            st = {}

            def q_piece(rb, hh):
                def run():
                    prow = pl.ds(pl.multiple_of(b * (RC // 2) + rb * 64, 64), 64)
                    qq = jnp.dot(_up(x_p[rb * 64:(rb + 1) * 64, :]), _up(wq_s[:, hh * 128:(hh + 1) * 128]),
                                 preferred_element_type=F32)
                    q_s[hh, prow, :] = _pk(qq.astype(BF16))
                return run

            def u_piece(q):
                def run():
                    ucat = jnp.concatenate(
                        [_up(kv_s[cg, i * 64:(i + 1) * 64, :]) for i in range(4 * q, 4 * q + 4)], axis=1)
                    u_s[:, q * 512:(q + 1) * 512] = jnp.dot(fh, ucat, preferred_element_type=F32)
                return run

            def h_piece(q):
                def run():
                    hcat = jnp.concatenate(
                        [h_s[cg, :, m * CB:(m + 1) * CB] for m in range(4 * q, 4 * q + 4)], axis=0)
                    st["hh", q] = lax.dot_general(fh, hcat, NT, preferred_element_type=F32)
                return run

            sgn = jnp.where((lax.broadcasted_iota(jnp.int32, (64, 128), 0) & 1) == 0,
                            1.0, -1.0).astype(F32)

            def t_step(m):
                def run():
                    cur = st["hh", m // 4][:, (m % 4) * CB:(m % 4 + 1) * CB]
                    tr = sgn * cur[64:128]
                    ti = sgn * cur[0:64]
                    if m > 0:
                        prv = st["hh", (m - 1) // 4][:, ((m - 1) % 4) * CB:((m - 1) % 4 + 1) * CB]
                        tr = prv[0:64] + tr
                        ti = prv[64:128] - ti
                    else:
                        ti = -ti
                    ht_s[0:64, m * CB:(m + 1) * CB] = tr
                    ht_s[64:128, m * CB:(m + 1) * CB] = ti
                return run

            RB = 32

            def p_step(i, rb, m):
                def run():
                    a0 = (i - m) * CB
                    b0 = m * CB
                    ur = u_s[rb:rb + RB, a0:a0 + CB]
                    ui = u_s[64 + rb:64 + rb + RB, a0:a0 + CB]
                    hr = ht_s[rb:rb + RB, b0:b0 + CB]
                    hi = ht_s[64 + rb:64 + rb + RB, b0:b0 + CB]
                    pr = ur * hr - ui * hi
                    pi = ur * hi + ui * hr
                    if m > 0:
                        pr = st["yr"] + pr
                        pi = st["yi"] + pi
                    st["yr"], st["yi"] = pr, pi
                    if m == i:
                        st["Y", i, rb] = (pr.astype(BF16), pi.astype(BF16))
                return run

            def i_piece(q):
                def run():
                    blocks = []
                    for i in range(4 * q, 4 * q + 4):
                        parts = [st.pop(("Y", i, rb)) for rb in range(0, 64, RB)]
                        blocks.append(jnp.concatenate([t[0] for t in parts] + [t[1] for t in parts], axis=0))
                    st["yo", q] = jnp.dot(gh, jnp.concatenate(blocks, axis=1), preferred_element_type=F32)
                return run

            def y_step(i):
                def run():
                    yo = st["yo", i // 4][:, (i % 4) * CB:(i % 4 + 1) * CB]
                    old = jnp.where(hf == 0, 0.0, y_s[cg, i * CB:(i + 1) * CB, :])
                    y_s[cg, i * CB:(i + 1) * CB, :] = old + yo
                return run

            rsteps = [(lambda s=s, wh=wh: relayout_wkv_step(gn, b, s, wh)) for s in range(4) for wh in range(2)]
            for q in range(4):
                u_piece(q)()
            for q in range(4):
                h_piece(q)()
            qp = [q_piece(rb, hh) for rb in range(RC // 128) for hh in range(HG)]
            aux = [t_step(m) for m in range(NCB)]
            psteps = [(i, rb, m) for i in range(NCB) for rb in range(0, 64, RB) for m in range(i + 1)]
            NQ1 = 31
            per = len(psteps) / float(NQ1 - 1)
            done = 0
            pend_i = [0, 1, 2, 3]
            pend_y = []
            for k in range(len(qp)):
                qp[k]()
                if k % HG == HG - 1:
                    stage_x(bn, k // HG)
                if k == 0:
                    for a in aux:
                        a()
                    continue
                while pend_i and done >= 2 * sum(range(1, 4 * pend_i[0] + 5)) + (20 if pend_i[0] < 3 else 0):
                    q = pend_i.pop(0)
                    i_piece(q)()
                    pend_y += list(range(4 * q, 4 * q + 4))
                    break
                tgt = min(len(psteps), int(round(per * k)))
                while done < tgt:
                    p_step(*psteps[done])()
                    done += 1
                if k >= 1 and rsteps:
                    rsteps.pop(0)()
                ny = 1 if pend_i else 2
                for _ in range(ny):
                    if pend_y:
                        y_step(pend_y.pop(0))()
            assert not pend_i and not rsteps
            while pend_y:
                y_step(pend_y.pop(0))()
            return c2

        @pl.when(g + 1 < NG)
        def _():
            for cp in cp_kvaux(jnp.minimum(g + 1, NG - 1)):
                cp.start()
            cp_h(jnp.minimum(g + 1, NG - 1)).start()

        cp_h(g).wait()

        @pl.when(g == 0)
        def _():
            cp_x(0).wait()
            for rb in range(RC // 128):
                stage_x(0, rb)

        lax.fori_loop(0, NRC, q_body, 0)

        mask = (lax.broadcasted_iota(jnp.int32, (BQ, BQ), 1)
                <= lax.broadcasted_iota(jnp.int32, (BQ, BQ), 0))
        HB = BQ // 2

        def attn_body(t, c2):
            def qk(hh, i, z):
                q = q_s[hh, i * HB:(i + 1) * HB, :]
                if z is not None:
                    q = jnp.concatenate([q[0:8] + z, q[8:]], axis=0)
                return lax.dot_general(_up(q), _up(k_s[hh, 0:(i + 1) * HB, :]), NT,
                                       preferred_element_type=F32)

            def sm(i, s):
                L = (i + 1) * BQ
                sd = jnp.where(mask, s[:, L - BQ:], NEG)
                s = jnp.concatenate([s[:, :L - BQ], sd], axis=1) if i > 0 else sd
                m = jnp.max(s, axis=1, keepdims=True)
                p = jnp.exp2(s - m)
                l = jnp.sum(p, axis=1, keepdims=True)
                return p.astype(BF16), l

            def pv(hh, i, p):
                return jnp.dot(p, _up(v_s[hh, 0:(i + 1) * HB, :]), preferred_element_type=F32)

            def fin(hh, i, ctx, l):
                r = pl.reciprocal(l, approx=True)
                r = r * (2.0 - l * r)
                o = _pk((ctx * r).astype(BF16))
                ctx_s[g * HG + hh, i * HB:(i + 1) * HB, :] = o
                a = o[0:8]
                for kk in range(1, 8):
                    a = a | o[8 * kk:8 * kk + 8]
                return (a & 1) >> 1

            order = []
            for i in range(NBQ // 2):
                big, small = NBQ // 2 + i, (i + NBQ // 4) % (NBQ // 2)
                for u in range(0, AH, 2):
                    ha, hb = AH * t + u, AH * t + u + 1
                    order += [(ha, big), (hb, big), (hb, small), (ha, small)]
            n = len(order)
            lag = 3
            ss, cs, zs = {}, {}, {}
            ss[0] = qk(*order[0], None)
            for j in range(n + lag):
                if j + 1 < n:
                    ss[j + 1] = qk(*order[j + 1], zs.pop(j + 1, None))
                if j < n:
                    p, l = sm(order[j][1], ss.pop(j))
                    cs[j] = (pv(*order[j], p), l)
                if 0 <= j - lag < n:
                    zs[j + 2] = fin(*order[j - lag], *cs.pop(j - lag))
            return c2

        lax.fori_loop(0, HG // AH, attn_body, 0)
        return carry

    lax.fori_loop(0, NG, group_body, 0)

    cp_wo.wait()
    cp_small[1].wait()
    cp_small[2].wait()

    def out_body(r, carry):
        rows = pl.ds(pl.multiple_of(r * FO, FO), FO)
        prow = pl.ds(pl.multiple_of(r * (FO // 2), FO // 2), FO // 2)
        ctx = jnp.concatenate([_up(ctx_s[hh, prow, :]) for hh in range(H)], axis=1)
        a = jnp.dot(ctx, wo_v[...], preferred_element_type=F32)
        xf = x_v[rows, :].astype(F32)
        gw = gw_v[...].astype(F32)[None, :]
        gate = jax.nn.sigmoid(jnp.sum(xf * gw, axis=1, keepdims=True))
        dd = d_v[...].astype(F32)[None, :]
        for cg in range(NCG):
            cols = slice(cg * 128, (cg + 1) * 128)
            yb = y_s[cg, rows, :] + _up(kv_s[cg, prow, :]).astype(F32) * dd[:, cols]
            o_s[rows, cols] = (gate * a[:, cols] + (1.0 - gate) * (xf[:, cols] * yb)).astype(BF16)
        cp_o(r).start()
        return carry

    lax.fori_loop(0, S // FO, out_body, 0)
    for r in range(S // FO):
        cp_o(r).wait()


@jax.jit
def pallas_gated_mix__compressed_kv_cla__ssm_conv_h3__prompt_kernel(
    A_x: jax.Array,
    A_c_kv: jax.Array,
    A_w_q: jax.Array,
    A_w_uk: jax.Array,
    A_w_uv: jax.Array,
    A_w_o: jax.Array,
    B_q: jax.Array,
    B_k: jax.Array,
    B_v: jax.Array,
    B_shift_k: jax.Array,
    B_ssm_k: jax.Array,
    B_ssm_D: jax.Array,
    gate_w: jax.Array,
):
    del B_q
    x = A_x.reshape(S, M)
    c = A_c_kv.reshape(S, DC)
    wq = A_w_q.reshape(M, NG, HG, D)
    wuk = A_w_uk.reshape(DC, NG, HG, D)
    wuv = A_w_uv.reshape(DC, NG, HG, D)
    wo = A_w_o.reshape(H * D, M)
    bk = B_k.reshape(S, M)
    bv = B_v.reshape(S, M)
    skt = B_shift_k.T
    hk = B_ssm_k.reshape(NCG, 128, S)

    dma = pltpu.SemaphoreType.DMA
    scratch = [
        pltpu.VMEM((S, M), BF16),
        pltpu.VMEM((S, DC), BF16),
        pltpu.VMEM((NG, M, HG, D), BF16),
        pltpu.VMEM((NG, DC, HG, D), BF16),
        pltpu.VMEM((NG, DC, HG, D), BF16),
        pltpu.VMEM((H * D, M), BF16),
        pltpu.VMEM((NCG, PADK + S, 128), BF16),
        pltpu.VMEM((NCG, S, 128), BF16),
        pltpu.VMEM((NCG, 128, S), BF16),
        pltpu.VMEM((RC // 2, M), U32),
        pltpu.VMEM((RC // 2, DC), U32),
        pltpu.VMEM((M // 2, HG * D), U32),
        pltpu.VMEM((DC // 2, 2 * HG * D), U32),
        pltpu.VMEM((HG, S // 2, D), U32),
        pltpu.VMEM((HG, S // 2, D), U32),
        pltpu.VMEM((HG, S // 2, D), U32),
        pltpu.VMEM((H, S // 2, D), U32),
        pltpu.VMEM((NCG, S // 2, 128), U32),
        pltpu.VMEM((NCG, S, 128), F32),
        pltpu.VMEM((128, S), F32),
        pltpu.VMEM((128, S), F32),
        pltpu.VMEM((2, 64, 128), U32),
        pltpu.VMEM((2, 64, 128), U32),
        pltpu.VMEM((S, M), BF16),
        pltpu.VMEM((4, M), BF16),
        pltpu.VMEM((M,), BF16),
        pltpu.VMEM((M,), BF16),
        dma((4,)), dma((4,)), dma((20,)), dma((NG * 8,)), dma((1,)), dma((NG,)), dma((3,)),
        dma((S // FO,)),
    ]
    out = pl.pallas_call(
        _kernel,
        out_shape=jax.ShapeDtypeStruct((S, M), BF16),
        in_specs=[pl.BlockSpec(memory_space=pl.ANY)] * 12,
        out_specs=pl.BlockSpec(memory_space=pl.ANY),
        scratch_shapes=scratch,
        compiler_params=pltpu.CompilerParams(vmem_limit_bytes=120 * 1024 * 1024),
    )(x, c, wq, wuk, wuv, wo, bk, bv, skt, hk, B_ssm_D, gate_w)
    return out.reshape(1, S, M)
```
